```python
import jax
import jax.numpy as jnp

def _softmax(x, axis=-1):
    return jax.nn.softmax(x, axis=axis)
def _gelu(x):
    return jax.nn.gelu(x, approximate=True)
def _silu(x):
    return jax.nn.silu(x)
def _sigmoid(x):
    return jax.nn.sigmoid(x)
def _layernorm(x, axis=-1, eps=1e-5):
    m = jnp.mean(x, axis=axis, keepdims=True)
    v = jnp.var(x, axis=axis, keepdims=True)
    return (x - m) / jnp.sqrt(v + eps)
def _scatter_add(tgt, idx, src, axis=0):
    return tgt.at[idx].add(src)
def _segment_sum(src, seg, n):
    return jax.ops.segment_sum(src, seg, n)
class _Rng:
    def __init__(self, key):
        self._k = key
    def _next(self):
        self._k, sub = jax.random.split(self._k)
        return sub
    def normal(self, shape):
        return jax.random.normal(self._next(), shape, dtype=jnp.bfloat16)
    def randint(self, lo, hi, shape):
        return jax.random.randint(self._next(), shape, lo, hi, dtype=jnp.int32)
    def uniform(self, shape, lo=0.0, hi=1.0):
        return jax.random.uniform(self._next(), shape, jnp.bfloat16, lo, hi)
    def permutation(self, n):
        return jax.random.permutation(self._next(), n)


kernel_name = 'recurrent_scan__gqa_block_cached__moe_arch_mod__prompt'

def setup_inputs():
    _rng = _Rng(jax.random.key(int.from_bytes(__import__("os").urandom(4), "little")))
    _w = (lambda a: (lambda t: t.astype(jnp.bfloat16) if jnp.issubdtype(t.dtype, jnp.floating) else t)(jnp.asarray(a)))
    def _A_setup():
        B, Sq, D = 1, 2048, 576
        Hq, Hkv, Sk, Dh = 32, 16, 2048, 128
        assert Hq % Hkv == 0, (Hq, Hkv)
        return {
            "x": _w((lambda *s: _rng.normal(s) * 0.05)(B, Sq, D)),
            "k_cache": _w((lambda *s: _rng.normal(s) * 0.05)(B, Hkv, Sk, Dh)),
            "v_cache": _w((lambda *s: _rng.normal(s) * 0.05)(B, Hkv, Sk, Dh)),
            "wq": _w((lambda *s: _rng.normal(s) * 0.05)(D, Hq * Dh) * (D ** -0.5)),
            "wo": _w((lambda *s: _rng.normal(s) * 0.05)(Hq * Dh, D) * ((Hq * Dh) ** -0.5)),
        }
    _A_in = _A_setup()

    def _B_setup():
        B, S, D, F, C = 1, 2048, 576, 4608, 8
        return {
            "x": _w((lambda *s: _rng.normal(s) * 0.05)(B, S, D)),
            "w_r": _w((lambda *s: _rng.normal(s) * 0.05)(D)),
            "w_gate": _w((lambda *s: _rng.normal(s) * 0.05)(D, F)),
            "w_up": _w((lambda *s: _rng.normal(s) * 0.05)(D, F)),
            "w_down": _w((lambda *s: _rng.normal(s) * 0.05)(F, D)),
        }
    _B_in = _B_setup()

    return {
        "A_x": _A_in["x"],
        "A_k_cache": _A_in["k_cache"],
        "A_v_cache": _A_in["v_cache"],
        "A_wq": _A_in["wq"],
        "A_wo": _A_in["wo"],
        "B_x": _B_in["x"],
        "B_w_r": _B_in["w_r"],
        "B_w_gate": _B_in["w_gate"],
        "B_w_up": _B_in["w_up"],
        "B_w_down": _B_in["w_down"],
    }

def reference(A_x, A_k_cache, A_v_cache, A_wq, A_wo, B_x, B_w_r, B_w_gate, B_w_up, B_w_down):
    def _A_ref(x, k_cache, v_cache, wq, wo):
        B, Sq, D = x.shape
        Hq, Dh = 32, 128
        Hkv = k_cache.shape[1]
        rep = Hq // Hkv
        q = (lambda x, *d: x.transpose(*d))((x @ wq).reshape(B, Sq, Hq, Dh), 0, 2, 1, 3)
        k = jnp.repeat(k_cache, rep, axis=1)
        v = jnp.repeat(v_cache, rep, axis=1)
        scores = jnp.einsum("bhqd,bhkd->bhqk", q, k) * (Dh ** -0.5)
        p = _softmax(scores, axis=-1)
        o = jnp.einsum("bhqk,bhkd->bhqd", p, v)
        return (lambda x, *d: x.transpose(*d))(o, 0, 2, 1, 3).reshape(B, Sq, Hq * Dh) @ wo

    def _B_ref(x, w_r, w_gate, w_up, w_down):
        B, S, D = x.shape
        C = 8
        r = x @ w_r
        idx = jnp.argsort(-r, axis=-1)[:, :C]
        idx_e = jnp.repeat(idx.reshape(B, C, 1), D, axis=2)
        x_sel = jnp.take_along_axis(x, idx_e, axis=1)
        g = _silu(x_sel @ w_gate)
        u = x_sel @ w_up
        y = (g * u) @ w_down
        r_sel = _sigmoid(jnp.take_along_axis(r, idx, axis=1))
        y = y * r_sel.reshape(B, C, 1)
        b_off = (jnp.arange(B) * S).reshape(B, 1)
        flat_idx = (idx + b_off).reshape(B * C)
        zero = (x * 0.0).reshape(B * S, D)
        upd = _scatter_add(zero, flat_idx, y.reshape(B * C, D), axis=0)
        return x + upd.reshape(B, S, D)

    x = A_x
    xn = _layernorm(x, axis=-1)
    s = _A_ref(xn, A_k_cache, A_v_cache, A_wq, A_wo)
    g = _silu(_B_ref(xn, B_w_r, B_w_gate, B_w_up, B_w_down))
    return x + s * g
```

```python
import jax
import jax.numpy as jnp
from jax import lax
import jax.experimental.pallas as pl
import jax.experimental.pallas.tpu as pltpu

f32 = jnp.float32
bf16 = jnp.bfloat16

T = 2048
SK = 2048
DM = 576
DH = 128
HKV = 16
FF = 4608
CAP = 8
TT = 256
NSUB = T // TT
CK = 256
NC = SK // CK
NXP = 4
XP = T // NXP
EPS = 1e-5
QSCALE = 0.08837890625 * 1.4426950408889634
NT = (((1,), (1,)), ((), ()))

CFG = dict(qpos=5, opos=2)


def _rb(x):
    return x.astype(bf16).astype(f32)


def _sigmoid(x):
    return 0.5 * jnp.tanh(0.5 * x) + 0.5


def _silu(x):
    return x * _sigmoid(x)


def _kernel(xt_hbm, k_hbm, v_hbm, wq_hbm, wot_hbm, wr_ref, wg_hbm, wu_hbm, wdt_hbm,
            out_hbm,
            xt_ref, k_ref, v_ref, wq_ref, wot_ref, xn_ref, gt_ref, acc_ref, out_ref,
            qc_ref, sc_ref, oc_ref, xs_ref, rs_ref, idx_ref, wg_ref, wu_ref, wdt_ref,
            sem_x, sem_wq, sem_k, sem_v, sem_wo, sem_moe, sem_out):
    h = pl.program_id(0)
    qpos, opos = CFG['qpos'], CFG['opos']
    ncarry = 2 if qpos == 0 else 1

    def cp_x(part):
        cols = pl.ds(part * XP, XP)
        return pltpu.make_async_copy(xt_hbm.at[:, cols], xt_ref.at[:, cols], sem_x.at[part])

    def _hcols(hh):
        start = hh * (2 * DH)
        if not isinstance(hh, int):
            start = pl.multiple_of(start, 2 * DH)
        return pl.ds(start, 2 * DH)

    def cp_wq(hh):
        return pltpu.make_async_copy(wq_hbm.at[:, _hcols(hh)], wq_ref.at[hh], sem_wq.at[hh])

    def cp_wo(hh):
        return pltpu.make_async_copy(wot_hbm.at[:, _hcols(hh)], wot_ref.at[hh], sem_wo.at[hh])

    def cp_k(hh):
        return pltpu.make_async_copy(k_hbm.at[hh], k_ref.at[hh], sem_k.at[hh])

    def cp_v(hh):
        return pltpu.make_async_copy(v_hbm.at[hh], v_ref.at[hh], sem_v.at[hh])

    def cp_moe():
        return (pltpu.make_async_copy(wg_hbm, wg_ref, sem_moe.at[0]),
                pltpu.make_async_copy(wu_hbm, wu_ref, sem_moe.at[1]),
                pltpu.make_async_copy(wdt_hbm, wdt_ref, sem_moe.at[2]))

    def cp_out(t):
        cols = pl.ds(t * TT, TT)
        return pltpu.make_async_copy(out_ref.at[:, cols], out_hbm.at[:, cols], sem_out.at[t])

    def layernorm_tile(t, wr_col):
        cols = slice(t * TT, (t + 1) * TT)
        x = xt_ref[:, cols].astype(f32)
        mean = jnp.sum(x, axis=0, keepdims=True) * (1.0 / DM)
        xc = x - mean
        var = jnp.sum(xc * xc, axis=0, keepdims=True) * (1.0 / DM)
        den = _rb(jnp.sqrt(_rb(_rb(var) + EPS)))
        xn = _rb(_rb(x - _rb(mean)) * (1.0 / den))
        xn_ref[cols, :] = xn.T.astype(bf16)
        gt_ref[:, cols] = _silu(xn).astype(bf16)
        acc_ref[:, cols] = jnp.zeros((DM, TT), f32)
        wr2 = jnp.concatenate([wr_col] * (TT // 128), axis=1)
        return jnp.sum(xn * wr2, axis=0, keepdims=True)

    def route(r):
        r = _rb(r)
        rbits = pltpu.bitcast(r, jnp.int32) >> 16
        mono = jnp.where(rbits < 0, -(rbits & 0x7FFF), rbits)
        lane = lax.broadcasted_iota(jnp.int32, (1, T), 1)
        keys = mono * T + (T - 1 - lane)
        sub = lax.broadcasted_iota(jnp.int32, (16, DM), 0)
        for j in range(CAP):
            kmax = jnp.max(keys)
            sel = keys == kmax
            keys = jnp.where(sel, jnp.iinfo(jnp.int32).min, keys)
            idx = (T - 1) - (kmax & (T - 1))
            idx_ref[j] = idx
            rs_ref[j:j + 1, :] = jnp.broadcast_to(
                jnp.sum(jnp.where(sel, r, 0.0), axis=-1, keepdims=True), (1, 128))
            blk = xn_ref[pl.ds(pl.multiple_of((idx >> 4) << 4, 16), 16), :].astype(f32)
            xs_ref[j:j + 1, :] = jnp.sum(jnp.where(sub == (idx & 15), blk, 0.0), axis=0, keepdims=True)

    def expert():
        xs32 = xs_ref[...]
        xs = xs32.astype(bf16)
        gate = _rb(_silu(_rb(jnp.dot(xs, wg_ref[...], preferred_element_type=f32))))
        up = _rb(jnp.dot(xs, wu_ref[...], preferred_element_type=f32))
        y = _rb(lax.dot_general((gate * up).astype(bf16), wdt_ref[...], NT, preferred_element_type=f32))
        rs = _rb(_sigmoid(rs_ref[:, 0:1]))
        y = _rb(y * rs)
        gnew = _silu(_rb(xs32 + y))
        gnew_t = jnp.concatenate([gnew, jnp.zeros((128 - CAP, DM), f32)], axis=0).T
        lane128 = lax.broadcasted_iota(jnp.int32, (DM, 128), 1)
        for j in range(CAP):
            i = idx_ref[j]
            blk = pl.ds(pl.multiple_of((i >> 7) << 7, 128), 128)
            col = jnp.broadcast_to(gnew_t[:, j:j + 1], (DM, 128))
            old = gt_ref[:, blk].astype(f32)
            gt_ref[:, blk] = jnp.where(lane128 == (i & 127), col, old).astype(bf16)

    def qproj(t, w):
        q = jnp.dot(xn_ref[t * TT:(t + 1) * TT, :], w, preferred_element_type=f32) * QSCALE
        q = q.astype(bf16)
        return jnp.concatenate([q[:, :DH], q[:, DH:]], axis=0)

    def qk(q, hh, c):
        return lax.dot_general(q, k_ref[hh, c * CK:(c + 1) * CK, :], NT, preferred_element_type=f32)

    def finalize(lp, o):
        l = jnp.sum(lp, axis=-1, keepdims=True)
        r0 = pl.reciprocal(l, approx=True)
        r = r0 * (2.0 - l * r0)
        o = (o * r).astype(bf16)
        return jnp.concatenate([o[:TT], o[TT:]], axis=1)

    def oproj(o, w):
        return lax.dot_general(w, o, NT, preferred_element_type=f32)

    def attention_step():
        hn = jnp.minimum(h + 1, HKV - 1)
        hp = jnp.maximum(h - 1, 0)
        q, sc, st, fin = {}, {}, {}, {}
        for j in range(ncarry):
            q[j] = qc_ref[j]
        sc[(0, 0)] = sc_ref[...]
        fin[-1] = oc_ref[...]

        def pv(t, c):
            s = sc.pop((t, c))
            mc = jnp.max(s, axis=-1, keepdims=True)
            vc = v_ref[h, c * CK:(c + 1) * CK, :]
            if c == 0:
                m = mc
                p = jnp.exp2(s - m)
                lp = p[:, 0:128]
                for j in range(1, CK // 128):
                    lp = lp + p[:, j * 128:(j + 1) * 128]
                o = jnp.dot(p.astype(bf16), vc, preferred_element_type=f32)
            else:
                m0, lp0, o0 = st[t]
                m = jnp.maximum(m0, mc)
                a = jnp.exp2(m0 - m)
                p = jnp.exp2(s - m)
                lp = lp0 * a
                for j in range(CK // 128):
                    lp = lp + p[:, j * 128:(j + 1) * 128]
                o = o0 * a + jnp.dot(p.astype(bf16), vc, preferred_element_type=f32)
            st[t] = (m, lp, o)
            if c == NC - 1:
                del st[t]
                if t == NSUB - 1:
                    oc_ref[...] = finalize(lp, o)
                else:
                    fin[t] = finalize(lp, o)

        items = [(t, c) for t in range(NSUB) for c in range(NC)]
        n = len(items)
        for i in range(n):
            t1, c1 = items[i + 1] if i + 1 < n else (NSUB, 0)
            if t1 < NSUB:
                sc[(t1, c1)] = qk(q[t1], h, c1)
            else:
                sc_ref[...] = qk(q[t1], hn, 0)
            if c1 == qpos:
                tq = t1 + 1
                if tq < NSUB:
                    q[tq] = qproj(tq, wq_ref[h])
                else:
                    q[tq] = qproj(tq - NSUB, wq_ref[hn])
                    qc_ref[tq - NSUB] = q[tq]
            t, c = items[i]
            pv(t, c)
            if c == opos:
                tp = (t - 1) % NSUB
                w = wot_ref[hp] if t == 0 else wot_ref[h]
                acc_ref[:, tp * TT:(tp + 1) * TT] += oproj(fin.pop(t - 1), w)

    @pl.when(h == 0)
    def _prologue():
        for p in range(NXP):
            cp_x(p).start()
        cp_wq(0).start()
        cp_k(0).start()
        cp_v(0).start()
        cp_wo(0).start()
        cp_wq(1).start()
        cp_k(1).start()
        wr_col = jnp.broadcast_to(wr_ref[...].astype(f32), (128, DM)).T
        oc_ref[...] = jnp.zeros((TT, 2 * DH), bf16)
        rparts = []
        for t in range(NSUB):
            if (t * TT) % XP == 0:
                cp_x(t * TT // XP).wait()
            if t == NSUB - 2:
                cp_wq(0).wait()
                cp_k(0).wait()
            rparts.append(layernorm_tile(t, wr_col))
        route(jnp.concatenate(rparts, axis=1))
        for j in range(ncarry):
            qj = qproj(j, wq_ref[0])
            qc_ref[j] = qj
            if j == 0:
                sc_ref[...] = qk(qj, 0, 0)

    @pl.when(h > 0)
    def _():
        cp_v(h).wait()
        cp_wo(h).wait()

    @pl.when(h == 0)
    def _():
        cp_v(0).wait()
        cp_wo(0).wait()

    @pl.when(h + 1 < HKV)
    def _():
        cp_wq(h + 1).wait()
        cp_k(h + 1).wait()
        cp_v(h + 1).start()
        cp_wo(h + 1).start()

    @pl.when(h + 2 < HKV)
    def _():
        cp_wq(h + 2).start()
        cp_k(h + 2).start()

    @pl.when(h == 0)
    def _():
        for c in cp_moe():
            c.start()

    @pl.when(h == 2)
    def _():
        for c in cp_moe():
            c.wait()
        expert()

    attention_step()

    @pl.when(h == HKV - 1)
    def _epilogue():
        tl = NSUB - 1
        for t in range(NSUB):
            cols = slice(t * TT, (t + 1) * TT)
            s = acc_ref[:, cols]
            if t == tl:
                s = s + oproj(oc_ref[...], wot_ref[HKV - 1])
            out_ref[:, cols] = (xt_ref[:, cols].astype(f32)
                                + s * gt_ref[:, cols].astype(f32)).astype(bf16)
            cp_out(t).start()
        for t in range(NSUB):
            cp_out(t).wait()


@jax.jit
def pallas_recurrent_scan__gqa_block_cached__moe_arch_mod__prompt_kernel(
    A_x: jax.Array,
    A_k_cache: jax.Array,
    A_v_cache: jax.Array,
    A_wq: jax.Array,
    A_wo: jax.Array,
    B_x: jax.Array,
    B_w_r: jax.Array,
    B_w_gate: jax.Array,
    B_w_up: jax.Array,
    B_w_down: jax.Array,
):
    del B_x
    xt = A_x.reshape(T, DM).T
    k = A_k_cache.reshape(HKV, SK, DH)
    v = A_v_cache.reshape(HKV, SK, DH)
    wot = A_wo.T
    wdt = B_w_down.T
    wr = B_w_r.reshape(1, DM)
    hbm = pl.BlockSpec(memory_space=pl.ANY)
    dma = pltpu.SemaphoreType.DMA
    out_t = pl.pallas_call(
        _kernel,
        out_shape=jax.ShapeDtypeStruct((DM, T), bf16),
        grid=(HKV,),
        in_specs=[hbm, hbm, hbm, hbm, hbm,
                  pl.BlockSpec((1, DM), lambda h: (0, 0)),
                  hbm, hbm, hbm],
        out_specs=hbm,
        scratch_shapes=[
            pltpu.VMEM((DM, T), bf16),
            pltpu.VMEM((HKV, SK, DH), bf16),
            pltpu.VMEM((HKV, SK, DH), bf16),
            pltpu.VMEM((HKV, DM, 2 * DH), bf16),
            pltpu.VMEM((HKV, DM, 2 * DH), bf16),
            pltpu.VMEM((T, DM), bf16),
            pltpu.VMEM((DM, T), bf16),
            pltpu.VMEM((DM, T), f32),
            pltpu.VMEM((DM, T), bf16),
            pltpu.VMEM((2, 2 * TT, DH), bf16),
            pltpu.VMEM((2 * TT, CK), f32),
            pltpu.VMEM((TT, 2 * DH), bf16),
            pltpu.VMEM((CAP, DM), f32),
            pltpu.VMEM((CAP, 128), f32),
            pltpu.SMEM((CAP,), jnp.int32),
            pltpu.VMEM((DM, FF), bf16),
            pltpu.VMEM((DM, FF), bf16),
            pltpu.VMEM((DM, FF), bf16),
            dma((NXP,)), dma((HKV,)), dma((HKV,)), dma((HKV,)), dma((HKV,)), dma((3,)), dma((NSUB,)),
        ],
        compiler_params=pltpu.CompilerParams(
            dimension_semantics=("arbitrary",),
            vmem_limit_bytes=120 * 1024 * 1024,
        ),
    )(xt, k, v, A_wq, wot, wr, B_w_gate, B_w_up, wdt)
    return out_t.T.reshape(1, T, DM)
```

```python
import jax
import jax.numpy as jnp
from jax import lax
import jax.experimental.pallas as pl
import jax.experimental.pallas.tpu as pltpu

f32 = jnp.float32
bf16 = jnp.bfloat16

T = 2048
SK = 2048
DM = 576
DH = 128
HKV = 16
FF = 4608
CAP = 8
TT = 256
NSUB = T // TT
CK = 256
NC = SK // CK
EPS = 1e-5
QSCALE = 0.08837890625 * 1.4426950408889634
NT = (((1,), (1,)), ((), ()))

QPOS = 5
OPOS = 3
PIECES = (2, 3, 3)
PSTART = tuple(sum(PIECES[:i]) for i in range(len(PIECES)))
WWAIT = 6
PAD0 = 4


def _rb(x):
    return x.astype(bf16).astype(f32)


def _sigmoid(x):
    return 0.5 * jnp.tanh(0.5 * x) + 0.5


def _silu(x):
    hx = 0.5 * x
    return hx + hx * jnp.tanh(hx)


def _kernel(xt_hbm, k_hbm, v_hbm, wq_hbm, wot_hbm, wr_hbm, wg_hbm, wu_hbm, wdt_hbm,
            out_hbm,
            pad_ref, xt_ref, k_ref, v_ref, wq_ref, wot_ref, xn_ref, gt_ref, acc_ref, out_ref,
            qc_ref, sc_ref, oc_ref, xs_ref, rs_ref, idx_ref, wg_ref, wu_ref, wdt_ref, wr_ref,
            sem_x, sem_r, sem_a, sem_b, sem_moe, sem_out):
    h = pl.program_id(0)

    def cp_x(part):
        cols = pl.ds(PSTART[part] * TT, PIECES[part] * TT)
        return pltpu.make_async_copy(xt_hbm.at[:, cols], xt_ref.at[:, cols], sem_x.at[part])

    def _hcols(hh):
        start = hh * (2 * DH)
        if not isinstance(hh, int):
            start = pl.multiple_of(start, 2 * DH)
        return pl.ds(start, 2 * DH)

    def grp_a(hh):
        first = pl.ds(0, CK)
        return (pltpu.make_async_copy(wq_hbm.at[:, _hcols(hh)], wq_ref.at[hh], sem_a.at[hh]),
                pltpu.make_async_copy(k_hbm.at[hh, first], k_ref.at[hh, first], sem_a.at[hh]))

    def grp_b(hh):
        rest = pl.ds(CK, SK - CK)
        return (pltpu.make_async_copy(k_hbm.at[hh, rest], k_ref.at[hh, rest], sem_b.at[hh]),
                pltpu.make_async_copy(v_hbm.at[hh], v_ref.at[hh], sem_b.at[hh]),
                pltpu.make_async_copy(wot_hbm.at[:, _hcols(hh)], wot_ref.at[hh], sem_b.at[hh]))

    def cp_moe():
        return (pltpu.make_async_copy(wg_hbm, wg_ref, sem_moe.at[0]),
                pltpu.make_async_copy(wu_hbm, wu_ref, sem_moe.at[1]),
                pltpu.make_async_copy(wdt_hbm, wdt_ref, sem_moe.at[2]))

    def cp_out(t):
        start = t * TT
        if not isinstance(t, int):
            start = pl.multiple_of(start, TT)
        cols = pl.ds(start, TT)
        return pltpu.make_async_copy(out_ref.at[:, cols], out_hbm.at[:, cols], sem_out.at[t])

    def layernorm_tile(t, wr8):
        cols = slice(t * TT, (t + 1) * TT)
        x = xt_ref[:, cols].astype(f32)
        mean = jnp.sum(x, axis=0, keepdims=True) * (1.0 / DM)
        mb = _rb(mean)
        d = x - mb
        dm = mean - mb
        var = jnp.sum(d * d, axis=0, keepdims=True) * (1.0 / DM) - dm * dm
        den = _rb(jnp.sqrt(_rb(_rb(var) + EPS)))
        y = _rb(d) * (1.0 / den)
        xb = y.astype(bf16)
        xn_ref[cols, :] = y.T.astype(bf16)
        gt_ref[:, cols] = _silu(xb.astype(f32))
        return jnp.dot(wr8, xb, preferred_element_type=f32)[0:1]

    def route(r):
        rbits = pltpu.bitcast(_rb(r), jnp.int32) >> 16
        mono = jnp.where(rbits < 0, -(rbits & 0x7FFF), rbits) + 32768
        lane = lax.broadcasted_iota(jnp.int32, (1, T), 1)
        keys = pltpu.bitcast(mono * T + (T - 1 - lane) + (1 << 23), f32)
        sub = lax.broadcasted_iota(jnp.int32, (16, DM), 0)
        for j in range(CAP):
            kv = jnp.max(keys, axis=1, keepdims=True)
            keys = jnp.where(keys == kv, 0.0, keys)
            ki = pltpu.bitcast(kv, jnp.int32) - (1 << 23)
            idx = (T - 1) - (ki[0, 0] & (T - 1))
            idx_ref[j] = idx
            code = (ki >> 11) - 32768
            bits = jnp.where(code < 0, (-code) | 0x8000, code) << 16
            rs_ref[j:j + 1, :] = jnp.broadcast_to(pltpu.bitcast(bits, f32), (1, 128))
            blk = xn_ref[pl.ds(pl.multiple_of((idx >> 4) << 4, 16), 16), :].astype(f32)
            xs_ref[j:j + 1, :] = jnp.sum(jnp.where(sub == (idx & 15), blk, 0.0), axis=0, keepdims=True)

    def expert():
        xs32 = xs_ref[...]
        xs = xs32.astype(bf16)
        gate = _rb(_silu(_rb(jnp.dot(xs, wg_ref[...], preferred_element_type=f32))))
        up = _rb(jnp.dot(xs, wu_ref[...], preferred_element_type=f32))
        y = _rb(lax.dot_general((gate * up).astype(bf16), wdt_ref[...], NT, preferred_element_type=f32))
        rs = _rb(_sigmoid(rs_ref[:, 0:1]))
        y = _rb(y * rs)
        gnew = _silu(_rb(xs32 + y))
        gnew_t = jnp.concatenate([gnew, jnp.zeros((128 - CAP, DM), f32)], axis=0).T
        lane128 = lax.broadcasted_iota(jnp.int32, (DM, 128), 1)
        for j in range(CAP):
            i = idx_ref[j]
            blk = pl.ds(pl.multiple_of((i >> 7) << 7, 128), 128)
            col = pltpu.roll(gnew_t, ((i & 127) + (128 - j)) & 127, 1)
            pltpu.store(gt_ref.at[:, blk], col, mask=lane128 == (i & 127))

    def qproj(t, w):
        q = jnp.dot(xn_ref[t * TT:(t + 1) * TT, :], w, preferred_element_type=f32) * QSCALE
        q = q.astype(bf16)
        return jnp.concatenate([q[:, :DH], q[:, DH:]], axis=0)

    def qk(q, hh, c):
        return lax.dot_general(q, k_ref[hh, c * CK:(c + 1) * CK, :], NT, preferred_element_type=f32)

    def finalize(lp, o):
        l = jnp.sum(lp, axis=-1, keepdims=True)
        r0 = pl.reciprocal(l, approx=True)
        r = r0 * (2.0 - l * r0)
        o = (o * r).astype(bf16)
        return jnp.concatenate([o[:TT], o[TT:]], axis=1)

    def oproj(o, w):
        return lax.dot_general(w, o, NT, preferred_element_type=f32)

    def attention_step():
        hn = jnp.minimum(h + 1, HKV - 1)
        hp = jnp.maximum(h - 1, 0)
        q, sc, st, fin = {0: qc_ref[...]}, {(0, 0): sc_ref[...]}, {}, {-1: oc_ref[...]}

        def pv(t, c):
            s = sc.pop((t, c))
            mc = jnp.max(s, axis=-1, keepdims=True)
            vc = v_ref[h, c * CK:(c + 1) * CK, :]
            if c == 0:
                m = mc
                p = jnp.exp2(s - m)
                lp = p[:, 0:128]
                for j in range(1, CK // 128):
                    lp = lp + p[:, j * 128:(j + 1) * 128]
                o = jnp.dot(p.astype(bf16), vc, preferred_element_type=f32)
            else:
                m0, lp0, o0 = st[t]
                m = jnp.maximum(m0, mc)
                a = jnp.exp2(m0 - m)
                p = jnp.exp2(s - m)
                lp = lp0 * a
                for j in range(CK // 128):
                    lp = lp + p[:, j * 128:(j + 1) * 128]
                o = o0 * a + jnp.dot(p.astype(bf16), vc, preferred_element_type=f32)
            st[t] = (m, lp, o)
            if c == NC - 1:
                del st[t]
                if t == NSUB - 1:
                    oc_ref[...] = finalize(lp, o)
                else:
                    fin[t] = finalize(lp, o)

        items = [(t, c) for t in range(NSUB) for c in range(NC)]
        n = len(items)
        for i in range(n):
            t1, c1 = items[i + 1] if i + 1 < n else (NSUB, 0)
            if t1 < NSUB:
                sc[(t1, c1)] = qk(q[t1], h, c1)
            else:
                sc_ref[...] = qk(q[t1], hn, 0)
            if c1 == QPOS:
                tq = t1 + 1
                if tq < NSUB:
                    q[tq] = qproj(tq, wq_ref[h])
                else:
                    q[tq] = qproj(0, wq_ref[hn])
                    qc_ref[...] = q[tq]
            t, c = items[i]
            pv(t, c)
            if c == OPOS:
                tp = (t - 1) % NSUB
                w = wot_ref[hp] if t == 0 else wot_ref[h]
                acc_ref[:, tp * TT:(tp + 1) * TT] += oproj(fin.pop(t - 1), w)

    @pl.when(h == 0)
    def _prologue():
        cp_r = pltpu.make_async_copy(wr_hbm, wr_ref, sem_r)
        stages = {0: [cp_x(2)] + list(grp_a(0)), 1: list(grp_b(0)), 2: list(grp_a(1))}
        for c in (cp_x(0), cp_r, cp_x(1)):
            c.start()
        acc_ref[...] = jnp.zeros((DM, T), f32)
        oc_ref[...] = jnp.zeros((TT, 2 * DH), bf16)
        pad_ref[0:8, :] = jnp.zeros((8, 128), f32)
        rparts = []
        for t in range(NSUB):
            if t in PSTART:
                cp_x(PSTART.index(t)).wait()
                if t == 0:
                    cp_r.wait()
                    wr8 = jnp.broadcast_to(wr_ref[...].reshape(1, DM), (8, DM))
                for c in stages[PSTART.index(t)]:
                    c.start()
            if t == WWAIT:
                for c in grp_a(0):
                    c.wait()
            rparts.append(layernorm_tile(t, wr8))
        route(jnp.concatenate(rparts, axis=1))
        q0 = qproj(0, wq_ref[0])
        qc_ref[...] = q0
        sc_ref[...] = qk(q0, 0, 0)

    for c in grp_b(h):
        c.wait()

    @pl.when(h + 1 < HKV)
    def _():
        for c in grp_a(h + 1):
            c.wait()
        for c in grp_b(h + 1):
            c.start()

    @pl.when(h + 2 < HKV)
    def _():
        for c in grp_a(h + 2):
            c.start()

    @pl.when(h == 0)
    def _():
        for c in cp_moe():
            c.start()

    @pl.when(h == 2)
    def _():
        for c in cp_moe():
            c.wait()
        expert()

    attention_step()

    @pl.when(h == HKV - 1)
    def _epilogue():
        def combine(cols, s):
            out_ref[:, cols] = (xt_ref[:, cols].astype(f32) + s * gt_ref[:, cols]).astype(bf16)

        def body(t, carry):
            cols = pl.ds(pl.multiple_of(t * TT, TT), TT)
            combine(cols, acc_ref[:, cols])
            cp_out(t).start()
            return carry

        tl = NSUB - 1
        lax.fori_loop(0, tl, body, 0)
        cols = slice(tl * TT, T)
        combine(cols, acc_ref[:, cols] + oproj(oc_ref[...], wot_ref[HKV - 1]))
        cp_out(tl).start()
        for t in range(NSUB):
            cp_out(t).wait()


@jax.jit
def pallas_recurrent_scan__gqa_block_cached__moe_arch_mod__prompt_kernel(
    A_x: jax.Array,
    A_k_cache: jax.Array,
    A_v_cache: jax.Array,
    A_wq: jax.Array,
    A_wo: jax.Array,
    B_x: jax.Array,
    B_w_r: jax.Array,
    B_w_gate: jax.Array,
    B_w_up: jax.Array,
    B_w_down: jax.Array,
):
    del B_x
    xt = A_x.reshape(T, DM).T
    k = A_k_cache.reshape(HKV, SK, DH)
    v = A_v_cache.reshape(HKV, SK, DH)
    wot = A_wo.T
    wdt = B_w_down.T
    hbm = pl.BlockSpec(memory_space=pl.ANY)
    dma = pltpu.SemaphoreType.DMA
    out_t = pl.pallas_call(
        _kernel,
        out_shape=jax.ShapeDtypeStruct((DM, T), bf16),
        grid=(HKV,),
        in_specs=[hbm] * 9,
        out_specs=hbm,
        scratch_shapes=[
            pltpu.VMEM((8 * PAD0, 128), f32),
            pltpu.VMEM((DM, T), bf16),
            pltpu.VMEM((HKV, SK, DH), bf16),
            pltpu.VMEM((HKV, SK, DH), bf16),
            pltpu.VMEM((HKV, DM, 2 * DH), bf16),
            pltpu.VMEM((HKV, DM, 2 * DH), bf16),
            pltpu.VMEM((T, DM), bf16),
            pltpu.VMEM((DM, T), f32),
            pltpu.VMEM((DM, T), f32),
            pltpu.VMEM((DM, T), bf16),
            pltpu.VMEM((2 * TT, DH), bf16),
            pltpu.VMEM((2 * TT, CK), f32),
            pltpu.VMEM((TT, 2 * DH), bf16),
            pltpu.VMEM((CAP, DM), f32),
            pltpu.VMEM((CAP, 128), f32),
            pltpu.SMEM((CAP,), jnp.int32),
            pltpu.VMEM((DM, FF), bf16),
            pltpu.VMEM((DM, FF), bf16),
            pltpu.VMEM((DM, FF), bf16),
            pltpu.VMEM((DM,), bf16),
            dma((len(PIECES),)), dma(()), dma((HKV,)), dma((HKV,)), dma((3,)), dma((NSUB,)),
        ],
        compiler_params=pltpu.CompilerParams(
            dimension_semantics=("arbitrary",),
            disable_bounds_checks=True,
            vmem_limit_bytes=120 * 1024 * 1024,
        ),
    )(xt, k, v, A_wq, wot, B_w_r, B_w_gate, B_w_up, wdt)
    return out_t.T.reshape(1, T, DM)
```

```python
import jax
import jax.numpy as jnp
from jax import lax
import jax.experimental.pallas as pl
import jax.experimental.pallas.tpu as pltpu

f32 = jnp.float32
bf16 = jnp.bfloat16

T = 2048
SK = 2048
DM = 576
DH = 128
HKV = 16
FF = 4608
CAP = 8
TT = 256
NSUB = T // TT
CK = 256
NC = SK // CK
EPS = 1e-5
QSCALE = 0.08837890625 * 1.4426950408889634
NT = (((1,), (1,)), ((), ()))

QPOS = 5
OPOS = 3
PIECES = (2, 2, 2, 2)
PSTART = tuple(sum(PIECES[:i]) for i in range(len(PIECES)))
WWAIT = 6
PAD0 = 4


def _rb(x):
    return x.astype(bf16).astype(f32)


def _sigmoid(x):
    return 0.5 * jnp.tanh(0.5 * x) + 0.5


def _silu(x):
    hx = 0.5 * x
    return hx + hx * jnp.tanh(hx)


def _kernel(xt_hbm, k_hbm, v_hbm, wq_hbm, wot_hbm, wr_hbm, wg_hbm, wu_hbm, wdt_hbm,
            out_hbm,
            pad_ref, xt_ref, k_ref, v_ref, wq_ref, wot_ref, xn_ref, gt_ref, acc_ref, out_ref,
            qc_ref, sc_ref, oc_ref, xs_ref, rs_ref, idx_ref, wg_ref, wu_ref, wdt_ref, wr_ref,
            sem_x, sem_r, sem_a, sem_b, sem_moe, sem_out):
    h = pl.program_id(0)

    def cp_x(part):
        cols = pl.ds(PSTART[part] * TT, PIECES[part] * TT)
        return pltpu.make_async_copy(xt_hbm.at[:, cols], xt_ref.at[:, cols], sem_x.at[part])

    def _hcols(hh):
        start = hh * (2 * DH)
        if not isinstance(hh, int):
            start = pl.multiple_of(start, 2 * DH)
        return pl.ds(start, 2 * DH)

    def grp_a(hh):
        first = pl.ds(0, CK)
        return (pltpu.make_async_copy(wq_hbm.at[:, _hcols(hh)], wq_ref.at[hh], sem_a.at[hh]),
                pltpu.make_async_copy(k_hbm.at[hh, first], k_ref.at[hh, first], sem_a.at[hh]))

    def grp_b(hh):
        rest = pl.ds(CK, SK - CK)
        return (pltpu.make_async_copy(k_hbm.at[hh, rest], k_ref.at[hh, rest], sem_b.at[hh]),
                pltpu.make_async_copy(v_hbm.at[hh], v_ref.at[hh], sem_b.at[hh]),
                pltpu.make_async_copy(wot_hbm.at[:, _hcols(hh)], wot_ref.at[hh], sem_b.at[hh]))

    def cp_moe():
        return (pltpu.make_async_copy(wg_hbm, wg_ref, sem_moe.at[0]),
                pltpu.make_async_copy(wu_hbm, wu_ref, sem_moe.at[1]),
                pltpu.make_async_copy(wdt_hbm, wdt_ref, sem_moe.at[2]))

    def cp_out(t):
        start = t * TT
        if not isinstance(t, int):
            start = pl.multiple_of(start, TT)
        cols = pl.ds(start, TT)
        return pltpu.make_async_copy(out_ref.at[:, cols], out_hbm.at[:, cols], sem_out.at[t])

    def layernorm_tile(t, wr8):
        cols = slice(t * TT, (t + 1) * TT)
        x = xt_ref[:, cols].astype(f32)
        mean = jnp.sum(x, axis=0, keepdims=True) * (1.0 / DM)
        mb = _rb(mean)
        d = x - mb
        dm = mean - mb
        var = jnp.sum(d * d, axis=0, keepdims=True) * (1.0 / DM) - dm * dm
        den = _rb(jnp.sqrt(_rb(_rb(var) + EPS)))
        y = _rb(d) * (1.0 / den)
        xb = y.astype(bf16)
        xn = xb.astype(f32)
        xn_ref[cols, :] = xn.T
        gt_ref[:, cols] = _silu(xn)
        return jnp.dot(wr8, xb, preferred_element_type=f32)[0:1]

    def route(r):
        rbits = pltpu.bitcast(_rb(r), jnp.int32) >> 16
        mono = jnp.where(rbits < 0, -(rbits & 0x7FFF), rbits) + 32768
        lane = lax.broadcasted_iota(jnp.int32, (1, T), 1)
        keys = pltpu.bitcast(mono * T + (T - 1 - lane) + (1 << 23), f32)
        for j in range(CAP):
            kv = jnp.max(keys, axis=1, keepdims=True)
            keys = jnp.where(keys == kv, 0.0, keys)
            ki = pltpu.bitcast(kv, jnp.int32) - (1 << 23)
            idx = (T - 1) - (ki[0, 0] & (T - 1))
            idx_ref[j] = idx
            code = (ki >> 11) - 32768
            bits = jnp.where(code < 0, (-code) | 0x8000, code) << 16
            rs_ref[j:j + 1, :] = jnp.broadcast_to(pltpu.bitcast(bits, f32), (1, 128))
            xs_ref[j:j + 1, :] = xn_ref[pl.ds(idx, 1), :]

    def expert():
        xs32 = xs_ref[...]
        xs = xs32.astype(bf16)
        gate = _rb(_silu(_rb(jnp.dot(xs, wg_ref[...], preferred_element_type=f32))))
        up = _rb(jnp.dot(xs, wu_ref[...], preferred_element_type=f32))
        y = _rb(lax.dot_general((gate * up).astype(bf16), wdt_ref[...], NT, preferred_element_type=f32))
        rs = _rb(_sigmoid(rs_ref[:, 0:1]))
        y = _rb(y * rs)
        gnew = _silu(_rb(xs32 + y))
        gnew_t = jnp.concatenate([gnew, jnp.zeros((128 - CAP, DM), f32)], axis=0).T
        lane128 = lax.broadcasted_iota(jnp.int32, (DM, 128), 1)
        for j in range(CAP):
            i = idx_ref[j]
            blk = pl.ds(pl.multiple_of((i >> 7) << 7, 128), 128)
            col = pltpu.roll(gnew_t, ((i & 127) + (128 - j)) & 127, 1)
            pltpu.store(gt_ref.at[:, blk], col, mask=lane128 == (i & 127))

    def qproj(t, w):
        xn = xn_ref[t * TT:(t + 1) * TT, :].astype(bf16)
        q = jnp.dot(xn, w, preferred_element_type=f32) * QSCALE
        q = q.astype(bf16)
        return jnp.concatenate([q[:, :DH], q[:, DH:]], axis=0)

    def qk(q, hh, c):
        return lax.dot_general(q, k_ref[hh, c * CK:(c + 1) * CK, :], NT, preferred_element_type=f32)

    def finalize(lp, o):
        l = jnp.sum(lp, axis=-1, keepdims=True)
        r0 = pl.reciprocal(l, approx=True)
        r = r0 * (2.0 - l * r0)
        o = (o * r).astype(bf16)
        return jnp.concatenate([o[:TT], o[TT:]], axis=1)

    def oproj(o, w):
        return lax.dot_general(w, o, NT, preferred_element_type=f32)

    def attention_step():
        hn = jnp.minimum(h + 1, HKV - 1)
        hp = jnp.maximum(h - 1, 0)
        q, sc, st, fin = {0: qc_ref[...]}, {(0, 0): sc_ref[...]}, {}, {-1: oc_ref[...]}

        def pv(t, c):
            s = sc.pop((t, c))
            mc = jnp.max(s, axis=-1, keepdims=True)
            vc = v_ref[h, c * CK:(c + 1) * CK, :]
            if c == 0:
                m = mc
                p = jnp.exp2(s - m)
                lp = p[:, 0:128]
                for j in range(1, CK // 128):
                    lp = lp + p[:, j * 128:(j + 1) * 128]
                o = jnp.dot(p.astype(bf16), vc, preferred_element_type=f32)
            else:
                m0, lp0, o0 = st[t]
                m = jnp.maximum(m0, mc)
                a = jnp.exp2(m0 - m)
                p = jnp.exp2(s - m)
                lp = lp0 * a
                for j in range(CK // 128):
                    lp = lp + p[:, j * 128:(j + 1) * 128]
                o = o0 * a + jnp.dot(p.astype(bf16), vc, preferred_element_type=f32)
            st[t] = (m, lp, o)
            if c == NC - 1:
                del st[t]
                if t == NSUB - 1:
                    oc_ref[...] = finalize(lp, o)
                else:
                    fin[t] = finalize(lp, o)

        items = [(t, c) for t in range(NSUB) for c in range(NC)]
        n = len(items)
        for i in range(n):
            t1, c1 = items[i + 1] if i + 1 < n else (NSUB, 0)
            if t1 < NSUB:
                sc[(t1, c1)] = qk(q[t1], h, c1)
            else:
                sc_ref[...] = qk(q[t1], hn, 0)
            if c1 == QPOS:
                tq = t1 + 1
                if tq < NSUB:
                    q[tq] = qproj(tq, wq_ref[h])
                else:
                    q[tq] = qproj(0, wq_ref[hn])
                    qc_ref[...] = q[tq]
            t, c = items[i]
            pv(t, c)
            if c == OPOS:
                tp = (t - 1) % NSUB
                w = wot_ref[hp] if t == 0 else wot_ref[h]
                acc_ref[:, tp * TT:(tp + 1) * TT] += oproj(fin.pop(t - 1), w)

    @pl.when(h == 0)
    def _prologue():
        cp_r = pltpu.make_async_copy(wr_hbm, wr_ref, sem_r)
        k_rest, v0, wo0 = grp_b(0)
        stages = {0: [cp_x(2)] + list(grp_a(0)), 1: [cp_x(3), v0], 2: [k_rest, wo0], 3: list(grp_a(1))}
        for c in (cp_x(0), cp_r, cp_x(1)):
            c.start()
        acc_ref[...] = jnp.zeros((DM, T), f32)
        oc_ref[...] = jnp.zeros((TT, 2 * DH), bf16)
        pad_ref[0:8, :] = jnp.zeros((8, 128), f32)
        rparts = []
        for t in range(NSUB):
            if t in PSTART:
                cp_x(PSTART.index(t)).wait()
                if t == 0:
                    cp_r.wait()
                    wr8 = jnp.broadcast_to(wr_ref[...].reshape(1, DM), (8, DM))
                for c in stages[PSTART.index(t)]:
                    c.start()
            if t == WWAIT:
                for c in grp_a(0):
                    c.wait()
            rparts.append(layernorm_tile(t, wr8))
        route(jnp.concatenate(rparts, axis=1))
        q0 = qproj(0, wq_ref[0])
        qc_ref[...] = q0
        sc_ref[...] = qk(q0, 0, 0)

    for c in grp_b(h):
        c.wait()

    @pl.when(h + 1 < HKV)
    def _():
        for c in grp_a(h + 1):
            c.wait()
        for c in grp_b(h + 1):
            c.start()

    @pl.when(h + 2 < HKV)
    def _():
        for c in grp_a(h + 2):
            c.start()

    @pl.when(h == 0)
    def _():
        for c in cp_moe():
            c.start()

    @pl.when(h == 2)
    def _():
        for c in cp_moe():
            c.wait()
        expert()

    attention_step()

    @pl.when(h == HKV - 1)
    def _epilogue():
        def combine(cols, s):
            out_ref[:, cols] = (xt_ref[:, cols].astype(f32) + s * gt_ref[:, cols]).astype(bf16)

        def body(t, carry):
            cols = pl.ds(pl.multiple_of(t * TT, TT), TT)
            combine(cols, acc_ref[:, cols])
            cp_out(t).start()
            return carry

        tl = NSUB - 1
        lax.fori_loop(0, tl, body, 0)
        cols = slice(tl * TT, T)
        combine(cols, acc_ref[:, cols] + oproj(oc_ref[...], wot_ref[HKV - 1]))
        cp_out(tl).start()
        for t in range(NSUB):
            cp_out(t).wait()


@jax.jit
def pallas_recurrent_scan__gqa_block_cached__moe_arch_mod__prompt_kernel(
    A_x: jax.Array,
    A_k_cache: jax.Array,
    A_v_cache: jax.Array,
    A_wq: jax.Array,
    A_wo: jax.Array,
    B_x: jax.Array,
    B_w_r: jax.Array,
    B_w_gate: jax.Array,
    B_w_up: jax.Array,
    B_w_down: jax.Array,
):
    del B_x
    xt = A_x.reshape(T, DM).T
    k = A_k_cache.reshape(HKV, SK, DH)
    v = A_v_cache.reshape(HKV, SK, DH)
    wot = A_wo.T
    wdt = B_w_down.T
    hbm = pl.BlockSpec(memory_space=pl.ANY)
    dma = pltpu.SemaphoreType.DMA
    out_t = pl.pallas_call(
        _kernel,
        out_shape=jax.ShapeDtypeStruct((DM, T), bf16),
        grid=(HKV,),
        in_specs=[hbm] * 9,
        out_specs=hbm,
        scratch_shapes=[
            pltpu.VMEM((8 * PAD0, 128), f32),
            pltpu.VMEM((DM, T), bf16),
            pltpu.VMEM((HKV, SK, DH), bf16),
            pltpu.VMEM((HKV, SK, DH), bf16),
            pltpu.VMEM((HKV, DM, 2 * DH), bf16),
            pltpu.VMEM((HKV, DM, 2 * DH), bf16),
            pltpu.VMEM((T, DM), f32),
            pltpu.VMEM((DM, T), f32),
            pltpu.VMEM((DM, T), f32),
            pltpu.VMEM((DM, T), bf16),
            pltpu.VMEM((2 * TT, DH), bf16),
            pltpu.VMEM((2 * TT, CK), f32),
            pltpu.VMEM((TT, 2 * DH), bf16),
            pltpu.VMEM((CAP, DM), f32),
            pltpu.VMEM((CAP, 128), f32),
            pltpu.SMEM((CAP,), jnp.int32),
            pltpu.VMEM((DM, FF), bf16),
            pltpu.VMEM((DM, FF), bf16),
            pltpu.VMEM((DM, FF), bf16),
            pltpu.VMEM((DM,), bf16),
            dma((len(PIECES),)), dma(()), dma((HKV,)), dma((HKV,)), dma((3,)), dma((NSUB,)),
        ],
        compiler_params=pltpu.CompilerParams(
            dimension_semantics=("arbitrary",),
            disable_bounds_checks=True,
            vmem_limit_bytes=120 * 1024 * 1024,
        ),
    )(xt, k, v, A_wq, wot, B_w_r, B_w_gate, B_w_up, wdt)
    return out_t.T.reshape(1, T, DM)
```

```python
import jax
import jax.numpy as jnp
from jax import lax
import jax.experimental.pallas as pl
import jax.experimental.pallas.tpu as pltpu

f32 = jnp.float32
bf16 = jnp.bfloat16

T = 2048
SK = 2048
DM = 576
DH = 128
HKV = 16
FF = 4608
CAP = 8
TT = 256
NSUB = T // TT
CK = 256
NC = SK // CK
EPS = 1e-5
QSCALE = 0.08837890625 * 1.4426950408889634
NT = (((1,), (1,)), ((), ()))

QPOS = 2
OPOS = 1
MROWS = 128
NMX = 4
PIECES = (2, 2, 2, 2)
PSTART = tuple(sum(PIECES[:i]) for i in range(len(PIECES)))
WWAIT = 6
PAD0 = 4


def _rb(x):
    return x.astype(bf16).astype(f32)


def _sigmoid(x):
    return 0.5 * jnp.tanh(0.5 * x) + 0.5


def _silu(x):
    hx = 0.5 * x
    return hx + hx * jnp.tanh(hx)


def _kernel(xt_hbm, k_hbm, v_hbm, wq_hbm, wot_hbm, wr_hbm, wg_hbm, wu_hbm, wdt_hbm,
            out_hbm,
            pad_ref, xt_ref, k_ref, v_ref, wq_ref, wot_ref, xn_ref, gt_ref, acc_ref, out_ref,
            qc_ref, sc_ref, mc_ref, oc_ref, xs_ref, rs_ref, idx_ref, wg_ref, wu_ref, wdt_ref, wr_ref,
            sem_x, sem_r, sem_a, sem_b, sem_moe, sem_out):
    h = pl.program_id(0)

    def cp_x(part):
        cols = pl.ds(PSTART[part] * TT, PIECES[part] * TT)
        return pltpu.make_async_copy(xt_hbm.at[:, cols], xt_ref.at[:, cols], sem_x.at[part])

    def _hcols(hh):
        start = hh * (2 * DH)
        if not isinstance(hh, int):
            start = pl.multiple_of(start, 2 * DH)
        return pl.ds(start, 2 * DH)

    def grp_a(hh):
        first = pl.ds(0, CK)
        return (pltpu.make_async_copy(wq_hbm.at[:, _hcols(hh)], wq_ref.at[hh], sem_a.at[hh]),
                pltpu.make_async_copy(k_hbm.at[hh, first], k_ref.at[hh, first], sem_a.at[hh]))

    def grp_b(hh):
        rest = pl.ds(CK, SK - CK)
        return (pltpu.make_async_copy(k_hbm.at[hh, rest], k_ref.at[hh, rest], sem_b.at[hh]),
                pltpu.make_async_copy(v_hbm.at[hh], v_ref.at[hh], sem_b.at[hh]),
                pltpu.make_async_copy(wot_hbm.at[:, _hcols(hh)], wot_ref.at[hh], sem_b.at[hh]))

    def cp_moe():
        return (pltpu.make_async_copy(wg_hbm, wg_ref, sem_moe.at[0]),
                pltpu.make_async_copy(wu_hbm, wu_ref, sem_moe.at[1]),
                pltpu.make_async_copy(wdt_hbm, wdt_ref, sem_moe.at[2]))

    def cp_out(t):
        start = t * TT
        if not isinstance(t, int):
            start = pl.multiple_of(start, TT)
        cols = pl.ds(start, TT)
        return pltpu.make_async_copy(out_ref.at[:, cols], out_hbm.at[:, cols], sem_out.at[t])

    def layernorm_tile(t, wr8):
        cols = slice(t * TT, (t + 1) * TT)
        x = xt_ref[:, cols].astype(f32)
        mean = jnp.sum(x, axis=0, keepdims=True) * (1.0 / DM)
        mb = _rb(mean)
        d = x - mb
        dm = mean - mb
        var = jnp.sum(d * d, axis=0, keepdims=True) * (1.0 / DM) - dm * dm
        den = _rb(jnp.sqrt(_rb(_rb(var) + EPS)))
        y = _rb(d) * (1.0 / den)
        xb = y.astype(bf16)
        xn = xb.astype(f32)
        xn_ref[cols, :] = xn.T
        gt_ref[:, cols] = _silu(xn)
        return jnp.dot(wr8, xb, preferred_element_type=f32)[0:1]

    def route(r):
        rbits = pltpu.bitcast(_rb(r), jnp.int32) >> 16
        mono = jnp.where(rbits < 0, -(rbits & 0x7FFF), rbits) + 32768
        lane = lax.broadcasted_iota(jnp.int32, (1, T), 1)
        keys = pltpu.bitcast(mono * T + (T - 1 - lane) + (1 << 23), f32)
        for j in range(CAP):
            kv = jnp.max(keys, axis=1, keepdims=True)
            keys = jnp.where(keys == kv, 0.0, keys)
            ki = pltpu.bitcast(kv, jnp.int32) - (1 << 23)
            idx = (T - 1) - (ki[0, 0] & (T - 1))
            idx_ref[j] = idx
            code = (ki >> 11) - 32768
            bits = jnp.where(code < 0, (-code) | 0x8000, code) << 16
            rs_ref[j:j + 1, :] = jnp.broadcast_to(pltpu.bitcast(bits, f32), (1, 128))
            xs_ref[j:j + 1, :] = xn_ref[pl.ds(idx, 1), :]

    def expert():
        xs32 = xs_ref[...]
        xs = xs32.astype(bf16)
        gate = _rb(_silu(_rb(jnp.dot(xs, wg_ref[...], preferred_element_type=f32))))
        up = _rb(jnp.dot(xs, wu_ref[...], preferred_element_type=f32))
        y = _rb(lax.dot_general((gate * up).astype(bf16), wdt_ref[...], NT, preferred_element_type=f32))
        rs = _rb(_sigmoid(rs_ref[:, 0:1]))
        y = _rb(y * rs)
        gnew = _silu(_rb(xs32 + y))
        gnew_t = jnp.concatenate([gnew, jnp.zeros((128 - CAP, DM), f32)], axis=0).T
        lane128 = lax.broadcasted_iota(jnp.int32, (DM, 128), 1)
        gnew_b = gnew_t.astype(bf16)
        row = lax.broadcasted_iota(jnp.int32, (128, 128), 0)
        colk = lax.broadcasted_iota(jnp.int32, (128, 128), 1)
        for j in range(CAP):
            i = idx_ref[j]
            blk = pl.ds(pl.multiple_of((i >> 7) << 7, 128), 128)
            if j < NMX:
                perm = jnp.where(jnp.logical_and(row == j, colk == (i & 127)), 1.0, 0.0).astype(bf16)
                col = jnp.dot(gnew_b, perm, preferred_element_type=f32)
            else:
                col = pltpu.roll(gnew_t, ((i & 127) + (128 - j)) & 127, 1)
            pltpu.store(gt_ref.at[:, blk], col, mask=lane128 == (i & 127))

    def qproj(t, w):
        xn = xn_ref[t * TT:(t + 1) * TT, :].astype(bf16)
        q = jnp.dot(xn, w, preferred_element_type=f32) * QSCALE
        q = q.astype(bf16)
        return jnp.concatenate([q[:, :DH], q[:, DH:]], axis=0)

    def qk(q, hh, c):
        return lax.dot_general(q, k_ref[hh, c * CK:(c + 1) * CK, :], NT, preferred_element_type=f32)

    def finalize(lp, o):
        l = jnp.sum(lp, axis=-1, keepdims=True)
        r0 = pl.reciprocal(l, approx=True)
        r = r0 * (2.0 - l * r0)
        o = (o * r).astype(bf16)
        return jnp.concatenate([o[:TT], o[TT:]], axis=1)

    def oproj(o, w):
        return lax.dot_general(w, o, NT, preferred_element_type=f32)

    def attention_step():
        hn = jnp.minimum(h + 1, HKV - 1)
        hp = jnp.maximum(h - 1, 0)
        q, sc, st, fin = {0: qc_ref[...]}, {(0, 0): sc_ref[...]}, {}, {-1: oc_ref[...]}

        def rowmax(s):
            return jnp.broadcast_to(jnp.max(s, axis=-1, keepdims=True), (s.shape[0], 128))

        def pv(t, c):
            s = sc.pop((t, c))
            vc = v_ref[h, c * CK:(c + 1) * CK, :]
            wide = t == 0
            if t == 0 and c == 0:
                mc = jnp.concatenate([mc_ref[...], rowmax(s[MROWS:])], axis=0)
            elif wide:
                mc = rowmax(s)
            else:
                mc = jnp.max(s, axis=-1, keepdims=True)

            def probs(m):
                if wide:
                    return jnp.concatenate([jnp.exp2(s[:, j * 128:(j + 1) * 128] - m)
                                            for j in range(CK // 128)], axis=1)
                return jnp.exp2(s - m)

            if c == 0:
                m = mc
                p = probs(m)
                lp = p[:, 0:128]
                for j in range(1, CK // 128):
                    lp = lp + p[:, j * 128:(j + 1) * 128]
                o = jnp.dot(p.astype(bf16), vc, preferred_element_type=f32)
            else:
                m0, lp0, o0 = st[t]
                m = jnp.maximum(m0, mc)
                a = jnp.exp2(m0 - m)
                p = probs(m)
                pvp = jnp.dot(p.astype(bf16), vc, preferred_element_type=f32)
                lp = lp0 * a
                for j in range(CK // 128):
                    lp = lp + p[:, j * 128:(j + 1) * 128]
                o = pvp + o0 * a
            st[t] = (m, lp, o)
            if c == NC - 1:
                del st[t]
                if t == NSUB - 1:
                    oc_ref[...] = finalize(lp, o)
                else:
                    fin[t] = finalize(lp, o)

        items = [(t, c) for t in range(NSUB) for c in range(NC)]
        n = len(items)
        for i in range(n):
            t1, c1 = items[i + 1] if i + 1 < n else (NSUB, 0)
            if t1 < NSUB:
                sc[(t1, c1)] = qk(q[t1], h, c1)
            else:
                s_next = qk(q[t1], hn, 0)
                sc_ref[...] = s_next
                mc_ref[...] = rowmax(s_next[0:MROWS])
            t, c = items[i]
            pv(t, c)
            if c == OPOS:
                tp = (t - 1) % NSUB
                w = wot_ref[hp] if t == 0 else wot_ref[h]
                acc_ref[:, tp * TT:(tp + 1) * TT] += oproj(fin.pop(t - 1), w)
            if c1 == QPOS:
                tq = t1 + 1
                if tq < NSUB:
                    q[tq] = qproj(tq, wq_ref[h])
                else:
                    q[tq] = qproj(0, wq_ref[hn])
                    qc_ref[...] = q[tq]

    @pl.when(h == 0)
    def _prologue():
        cp_r = pltpu.make_async_copy(wr_hbm, wr_ref, sem_r)
        k_rest, v0, wo0 = grp_b(0)
        stages = {0: [cp_x(2)] + list(grp_a(0)), 1: [cp_x(3), v0], 2: [k_rest, wo0], 3: list(grp_a(1))}
        for c in (cp_x(0), cp_r, cp_x(1)):
            c.start()
        acc_ref[...] = jnp.zeros((DM, T), f32)
        oc_ref[...] = jnp.zeros((TT, 2 * DH), bf16)
        pad_ref[0:8, :] = jnp.zeros((8, 128), f32)
        rparts = []
        for t in range(NSUB):
            if t in PSTART:
                cp_x(PSTART.index(t)).wait()
                if t == 0:
                    cp_r.wait()
                    wr8 = jnp.broadcast_to(wr_ref[...].reshape(1, DM), (8, DM))
                for c in stages[PSTART.index(t)]:
                    c.start()
            if t == WWAIT:
                for c in grp_a(0):
                    c.wait()
            rparts.append(layernorm_tile(t, wr8))
        route(jnp.concatenate(rparts, axis=1))
        q0 = qproj(0, wq_ref[0])
        qc_ref[...] = q0
        s0 = qk(q0, 0, 0)
        sc_ref[...] = s0
        mc_ref[...] = jnp.broadcast_to(jnp.max(s0[0:MROWS], axis=-1, keepdims=True), (MROWS, 128))

    for c in grp_b(h):
        c.wait()

    @pl.when(h + 1 < HKV)
    def _():
        for c in grp_a(h + 1):
            c.wait()
        for c in grp_b(h + 1):
            c.start()

    @pl.when(h + 2 < HKV)
    def _():
        for c in grp_a(h + 2):
            c.start()

    @pl.when(h == 0)
    def _():
        for c in cp_moe():
            c.start()

    @pl.when(h == 2)
    def _():
        for c in cp_moe():
            c.wait()
        expert()

    attention_step()

    @pl.when(h == HKV - 1)
    def _epilogue():
        def combine(cols, s):
            out_ref[:, cols] = (xt_ref[:, cols].astype(f32) + s * gt_ref[:, cols]).astype(bf16)

        def body(t, carry):
            cols = pl.ds(pl.multiple_of(t * TT, TT), TT)
            combine(cols, acc_ref[:, cols])
            cp_out(t).start()
            return carry

        tl = NSUB - 1
        lax.fori_loop(0, tl, body, 0)
        cols = slice(tl * TT, T)
        combine(cols, acc_ref[:, cols] + oproj(oc_ref[...], wot_ref[HKV - 1]))
        cp_out(tl).start()
        for t in range(NSUB):
            cp_out(t).wait()


@jax.jit
def pallas_recurrent_scan__gqa_block_cached__moe_arch_mod__prompt_kernel(
    A_x: jax.Array,
    A_k_cache: jax.Array,
    A_v_cache: jax.Array,
    A_wq: jax.Array,
    A_wo: jax.Array,
    B_x: jax.Array,
    B_w_r: jax.Array,
    B_w_gate: jax.Array,
    B_w_up: jax.Array,
    B_w_down: jax.Array,
):
    del B_x
    xt = A_x.reshape(T, DM).T
    k = A_k_cache.reshape(HKV, SK, DH)
    v = A_v_cache.reshape(HKV, SK, DH)
    wot = A_wo.T
    wdt = B_w_down.T
    hbm = pl.BlockSpec(memory_space=pl.ANY)
    dma = pltpu.SemaphoreType.DMA
    out_t = pl.pallas_call(
        _kernel,
        out_shape=jax.ShapeDtypeStruct((DM, T), bf16),
        grid=(HKV,),
        in_specs=[hbm] * 9,
        out_specs=hbm,
        scratch_shapes=[
            pltpu.VMEM((8 * PAD0, 128), f32),
            pltpu.VMEM((DM, T), bf16),
            pltpu.VMEM((HKV, SK, DH), bf16),
            pltpu.VMEM((HKV, SK, DH), bf16),
            pltpu.VMEM((HKV, DM, 2 * DH), bf16),
            pltpu.VMEM((HKV, DM, 2 * DH), bf16),
            pltpu.VMEM((T, DM), f32),
            pltpu.VMEM((DM, T), f32),
            pltpu.VMEM((DM, T), f32),
            pltpu.VMEM((DM, T), bf16),
            pltpu.VMEM((2 * TT, DH), bf16),
            pltpu.VMEM((2 * TT, CK), f32),
            pltpu.VMEM((MROWS, 128), f32),
            pltpu.VMEM((TT, 2 * DH), bf16),
            pltpu.VMEM((CAP, DM), f32),
            pltpu.VMEM((CAP, 128), f32),
            pltpu.SMEM((CAP,), jnp.int32),
            pltpu.VMEM((DM, FF), bf16),
            pltpu.VMEM((DM, FF), bf16),
            pltpu.VMEM((DM, FF), bf16),
            pltpu.VMEM((DM,), bf16),
            dma((len(PIECES),)), dma(()), dma((HKV,)), dma((HKV,)), dma((3,)), dma((NSUB,)),
        ],
        compiler_params=pltpu.CompilerParams(
            dimension_semantics=("arbitrary",),
            disable_bounds_checks=True,
            vmem_limit_bytes=120 * 1024 * 1024,
        ),
    )(xt, k, v, A_wq, wot, B_w_r, B_w_gate, B_w_up, wdt)
    return out_t.T.reshape(1, T, DM)
```

```python
import jax
import jax.numpy as jnp
from jax import lax
import jax.experimental.pallas as pl
import jax.experimental.pallas.tpu as pltpu

f32 = jnp.float32
bf16 = jnp.bfloat16

T = 2048
SK = 2048
DM = 576
DH = 128
HKV = 16
FF = 4608
CAP = 8
TT = 256
NSUB = T // TT
CK = 256
NC = SK // CK
EPS = 1e-5
QSCALE = 0.08837890625 * 1.4426950408889634
NT = (((1,), (1,)), ((), ()))

QPOS = 2
OPOS = 1
MROWS = 128
NMX = 4
PIECES = (2, 2, 2, 2)
PSTART = tuple(sum(PIECES[:i]) for i in range(len(PIECES)))
WWAIT = 6
PAD0 = 4


def _rb(x):
    return x.astype(bf16).astype(f32)


def _sigmoid(x):
    return 0.5 * jnp.tanh(0.5 * x) + 0.5


def _silu(x):
    hx = 0.5 * x
    return hx + hx * jnp.tanh(hx)


def _kernel(xt_hbm, k_hbm, v_hbm, wq_hbm, wot_hbm, wr_hbm, wg_hbm, wu_hbm, wdt_hbm,
            out_hbm,
            pad_ref, xt_ref, k_ref, v_ref, wq_ref, wot_ref, xn_ref, gt_ref, acc_ref, out_ref,
            qc_ref, sc_ref, mc_ref, oc_ref, xs_ref, rs_ref, idx_ref, wg_ref, wu_ref, wdt_ref, wr_ref,
            sem_x, sem_r, sem_a, sem_b, sem_moe, sem_out):
    h = pl.program_id(0)

    def cp_x(part):
        cols = pl.ds(PSTART[part] * TT, PIECES[part] * TT)
        return pltpu.make_async_copy(xt_hbm.at[:, cols], xt_ref.at[:, cols], sem_x.at[part])

    def _hcols(hh):
        start = hh * (2 * DH)
        if not isinstance(hh, int):
            start = pl.multiple_of(start, 2 * DH)
        return pl.ds(start, 2 * DH)

    def grp_a(hh):
        first = pl.ds(0, CK)
        return (pltpu.make_async_copy(wq_hbm.at[:, _hcols(hh)], wq_ref.at[hh], sem_a.at[hh]),
                pltpu.make_async_copy(k_hbm.at[hh, first], k_ref.at[hh, first], sem_a.at[hh]))

    def grp_b(hh):
        rest = pl.ds(CK, SK - CK)
        return (pltpu.make_async_copy(k_hbm.at[hh, rest], k_ref.at[hh, rest], sem_b.at[hh]),
                pltpu.make_async_copy(v_hbm.at[hh], v_ref.at[hh], sem_b.at[hh]),
                pltpu.make_async_copy(wot_hbm.at[:, _hcols(hh)], wot_ref.at[hh], sem_b.at[hh]))

    def cp_moe():
        return (pltpu.make_async_copy(wg_hbm, wg_ref, sem_moe.at[0]),
                pltpu.make_async_copy(wu_hbm, wu_ref, sem_moe.at[1]),
                pltpu.make_async_copy(wdt_hbm, wdt_ref, sem_moe.at[2]))

    def cp_out(t):
        cols = pl.ds(t * TT, TT)
        return pltpu.make_async_copy(out_ref.at[:, cols], out_hbm.at[:, cols], sem_out.at[t])

    def layernorm_tile(t, wr8):
        cols = slice(t * TT, (t + 1) * TT)
        x = xt_ref[:, cols].astype(f32)
        mean = jnp.sum(x, axis=0, keepdims=True) * (1.0 / DM)
        mb = _rb(mean)
        d = x - mb
        dm = mean - mb
        var = jnp.maximum(jnp.sum(d * d, axis=0, keepdims=True) * (1.0 / DM) - dm * dm, 0.0)
        den = _rb(jnp.sqrt(_rb(_rb(var) + EPS)))
        y = _rb(d) * (1.0 / den)
        xb = y.astype(bf16)
        xn = xb.astype(f32)
        xn_ref[cols, :] = xn.T
        gt_ref[:, cols] = _silu(xn)
        return jnp.dot(wr8, xb, preferred_element_type=f32)[0:1]

    def route(r):
        rbits = pltpu.bitcast(_rb(r), jnp.int32) >> 16
        mono = jnp.where(rbits < 0, -(rbits & 0x7FFF), rbits) + 32768
        lane = lax.broadcasted_iota(jnp.int32, (1, T), 1)
        keys = pltpu.bitcast(mono * T + (T - 1 - lane) + (1 << 23), f32)
        for j in range(CAP):
            kv = jnp.max(keys, axis=1, keepdims=True)
            keys = jnp.where(keys == kv, 0.0, keys)
            ki = pltpu.bitcast(kv, jnp.int32) - (1 << 23)
            idx = (T - 1) - (ki[0, 0] & (T - 1))
            idx_ref[j] = idx
            code = (ki >> 11) - 32768
            bits = jnp.where(code < 0, (-code) | 0x8000, code) << 16
            rs_ref[j:j + 1, :] = jnp.broadcast_to(pltpu.bitcast(bits, f32), (1, 128))
            xs_ref[j:j + 1, :] = xn_ref[pl.ds(idx, 1), :]

    def expert():
        xs32 = xs_ref[...]
        xs = xs32.astype(bf16)
        gate = _rb(_silu(_rb(jnp.dot(xs, wg_ref[...], preferred_element_type=f32))))
        up = _rb(jnp.dot(xs, wu_ref[...], preferred_element_type=f32))
        y = _rb(lax.dot_general((gate * up).astype(bf16), wdt_ref[...], NT, preferred_element_type=f32))
        rs = _rb(_sigmoid(rs_ref[:, 0:1]))
        y = _rb(y * rs)
        gnew = _silu(_rb(xs32 + y))
        gnew_t = jnp.concatenate([gnew, jnp.zeros((128 - CAP, DM), f32)], axis=0).T
        lane128 = lax.broadcasted_iota(jnp.int32, (DM, 128), 1)
        gnew_b = gnew_t.astype(bf16)
        row = lax.broadcasted_iota(jnp.int32, (128, 128), 0)
        colk = lax.broadcasted_iota(jnp.int32, (128, 128), 1)
        for j in range(CAP):
            i = idx_ref[j]
            blk = pl.ds(pl.multiple_of((i >> 7) << 7, 128), 128)
            if j < NMX:
                perm = jnp.where(jnp.logical_and(row == j, colk == (i & 127)), 1.0, 0.0).astype(bf16)
                col = jnp.dot(gnew_b, perm, preferred_element_type=f32)
            else:
                col = pltpu.roll(gnew_t, ((i & 127) + (128 - j)) & 127, 1)
            pltpu.store(gt_ref.at[:, blk], col, mask=lane128 == (i & 127))

    def qproj(t, w):
        xn = xn_ref[t * TT:(t + 1) * TT, :].astype(bf16)
        q = jnp.dot(xn, w, preferred_element_type=f32) * QSCALE
        q = q.astype(bf16)
        return jnp.concatenate([q[:, :DH], q[:, DH:]], axis=0)

    def qk(q, hh, c):
        return lax.dot_general(q, k_ref[hh, c * CK:(c + 1) * CK, :], NT, preferred_element_type=f32)

    def finalize(lp, o):
        l = jnp.sum(lp, axis=-1, keepdims=True)
        r0 = pl.reciprocal(l, approx=True)
        r = r0 * (2.0 - l * r0)
        o = (o * r).astype(bf16)
        return jnp.concatenate([o[:TT], o[TT:]], axis=1)

    def oproj(o, w):
        return lax.dot_general(w, o, NT, preferred_element_type=f32)

    def combine(cols, s):
        out_ref[:, cols] = (xt_ref[:, cols].astype(f32) + s * gt_ref[:, cols]).astype(bf16)

    def attention_step():
        hn = jnp.minimum(h + 1, HKV - 1)
        hp = jnp.maximum(h - 1, 0)
        q, sc, st, fin = {0: qc_ref[...]}, {(0, 0): sc_ref[...]}, {}, {-1: oc_ref[...]}

        def rowmax(s):
            return jnp.broadcast_to(jnp.max(s, axis=-1, keepdims=True), (s.shape[0], 128))

        def pv(t, c):
            s = sc.pop((t, c))
            vc = v_ref[h, c * CK:(c + 1) * CK, :]
            wide = t == 0
            if t == 0 and c == 0:
                mc = jnp.concatenate([mc_ref[...], rowmax(s[MROWS:])], axis=0)
            elif wide:
                mc = rowmax(s)
            else:
                mc = jnp.max(s, axis=-1, keepdims=True)

            def probs(m):
                if wide:
                    return jnp.concatenate([jnp.exp2(s[:, j * 128:(j + 1) * 128] - m)
                                            for j in range(CK // 128)], axis=1)
                return jnp.exp2(s - m)

            if c == 0:
                m = mc
                p = probs(m)
                lp = p[:, 0:128]
                for j in range(1, CK // 128):
                    lp = lp + p[:, j * 128:(j + 1) * 128]
                o = jnp.dot(p.astype(bf16), vc, preferred_element_type=f32)
            else:
                m0, lp0, o0 = st[t]
                m = jnp.maximum(m0, mc)
                a = jnp.exp2(m0 - m)
                p = probs(m)
                pvp = jnp.dot(p.astype(bf16), vc, preferred_element_type=f32)
                lp = lp0 * a
                for j in range(CK // 128):
                    lp = lp + p[:, j * 128:(j + 1) * 128]
                o = pvp + o0 * a
            st[t] = (m, lp, o)
            if c == NC - 1:
                del st[t]
                if t == NSUB - 1:
                    oc_ref[...] = finalize(lp, o)
                else:
                    fin[t] = finalize(lp, o)

        items = [(t, c) for t in range(NSUB) for c in range(NC)]
        n = len(items)
        for i in range(n):
            t1, c1 = items[i + 1] if i + 1 < n else (NSUB, 0)
            if t1 < NSUB:
                sc[(t1, c1)] = qk(q[t1], h, c1)
            else:
                s_next = qk(q[t1], hn, 0)
                sc_ref[...] = s_next
                mc_ref[...] = rowmax(s_next[0:MROWS])
            t, c = items[i]
            pv(t, c)
            if c == OPOS:
                tp = (t - 1) % NSUB
                w = wot_ref[hp] if t == 0 else wot_ref[h]
                cols = slice(tp * TT, (tp + 1) * TT)
                s_new = acc_ref[:, cols] + oproj(fin.pop(t - 1), w)
                acc_ref[:, cols] = s_new
                if t > 0:
                    combine(cols, s_new)

                    @pl.when(h == HKV - 1)
                    def _():
                        cp_out(tp).start()
            if c1 == QPOS:
                tq = t1 + 1
                if tq < NSUB:
                    q[tq] = qproj(tq, wq_ref[h])
                else:
                    q[tq] = qproj(0, wq_ref[hn])
                    qc_ref[...] = q[tq]

    @pl.when(h == 0)
    def _prologue():
        cp_r = pltpu.make_async_copy(wr_hbm, wr_ref, sem_r)
        k_rest, v0, wo0 = grp_b(0)
        stages = {0: [cp_x(2)] + list(grp_a(0)), 1: [cp_x(3), v0], 2: [k_rest, wo0], 3: list(grp_a(1))}
        for c in (cp_x(0), cp_r, cp_x(1)):
            c.start()
        acc_ref[...] = jnp.zeros((DM, T), f32)
        oc_ref[...] = jnp.zeros((TT, 2 * DH), bf16)
        pad_ref[0:8, :] = jnp.zeros((8, 128), f32)
        rparts = []
        for t in range(NSUB):
            if t in PSTART:
                cp_x(PSTART.index(t)).wait()
                if t == 0:
                    cp_r.wait()
                    wr8 = jnp.broadcast_to(wr_ref[...].reshape(1, DM), (8, DM))
                for c in stages[PSTART.index(t)]:
                    c.start()
            if t == WWAIT:
                for c in grp_a(0):
                    c.wait()
            rparts.append(layernorm_tile(t, wr8))
        route(jnp.concatenate(rparts, axis=1))
        q0 = qproj(0, wq_ref[0])
        qc_ref[...] = q0
        s0 = qk(q0, 0, 0)
        sc_ref[...] = s0
        mc_ref[...] = jnp.broadcast_to(jnp.max(s0[0:MROWS], axis=-1, keepdims=True), (MROWS, 128))

    for c in grp_b(h):
        c.wait()

    @pl.when(h + 1 < HKV)
    def _():
        for c in grp_a(h + 1):
            c.wait()
        for c in grp_b(h + 1):
            c.start()

    @pl.when(h + 2 < HKV)
    def _():
        for c in grp_a(h + 2):
            c.start()

    @pl.when(h == 0)
    def _():
        for c in cp_moe():
            c.start()

    @pl.when(h == 2)
    def _():
        for c in cp_moe():
            c.wait()
        expert()

    attention_step()

    @pl.when(h == HKV - 1)
    def _epilogue():
        tl = NSUB - 1
        cols = slice(tl * TT, T)
        combine(cols, acc_ref[:, cols] + oproj(oc_ref[...], wot_ref[HKV - 1]))
        cp_out(tl).start()
        for t in range(NSUB):
            cp_out(t).wait()


@jax.jit
def pallas_recurrent_scan__gqa_block_cached__moe_arch_mod__prompt_kernel(
    A_x: jax.Array,
    A_k_cache: jax.Array,
    A_v_cache: jax.Array,
    A_wq: jax.Array,
    A_wo: jax.Array,
    B_x: jax.Array,
    B_w_r: jax.Array,
    B_w_gate: jax.Array,
    B_w_up: jax.Array,
    B_w_down: jax.Array,
):
    del B_x
    xt = A_x.reshape(T, DM).T
    k = A_k_cache.reshape(HKV, SK, DH)
    v = A_v_cache.reshape(HKV, SK, DH)
    wot = A_wo.T
    wdt = B_w_down.T
    hbm = pl.BlockSpec(memory_space=pl.ANY)
    dma = pltpu.SemaphoreType.DMA
    out_t = pl.pallas_call(
        _kernel,
        out_shape=jax.ShapeDtypeStruct((DM, T), bf16),
        grid=(HKV,),
        in_specs=[hbm] * 9,
        out_specs=hbm,
        scratch_shapes=[
            pltpu.VMEM((8 * PAD0, 128), f32),
            pltpu.VMEM((DM, T), bf16),
            pltpu.VMEM((HKV, SK, DH), bf16),
            pltpu.VMEM((HKV, SK, DH), bf16),
            pltpu.VMEM((HKV, DM, 2 * DH), bf16),
            pltpu.VMEM((HKV, DM, 2 * DH), bf16),
            pltpu.VMEM((T, DM), f32),
            pltpu.VMEM((DM, T), f32),
            pltpu.VMEM((DM, T), f32),
            pltpu.VMEM((DM, T), bf16),
            pltpu.VMEM((2 * TT, DH), bf16),
            pltpu.VMEM((2 * TT, CK), f32),
            pltpu.VMEM((MROWS, 128), f32),
            pltpu.VMEM((TT, 2 * DH), bf16),
            pltpu.VMEM((CAP, DM), f32),
            pltpu.VMEM((CAP, 128), f32),
            pltpu.SMEM((CAP,), jnp.int32),
            pltpu.VMEM((DM, FF), bf16),
            pltpu.VMEM((DM, FF), bf16),
            pltpu.VMEM((DM, FF), bf16),
            pltpu.VMEM((DM,), bf16),
            dma((len(PIECES),)), dma(()), dma((HKV,)), dma((HKV,)), dma((3,)), dma((NSUB,)),
        ],
        compiler_params=pltpu.CompilerParams(
            dimension_semantics=("arbitrary",),
            disable_bounds_checks=True,
            vmem_limit_bytes=120 * 1024 * 1024,
        ),
    )(xt, k, v, A_wq, wot, B_w_r, B_w_gate, B_w_up, wdt)
    return out_t.T.reshape(1, T, DM)
```

```python
import jax
import jax.numpy as jnp
from jax import lax
import jax.experimental.pallas as pl
import jax.experimental.pallas.tpu as pltpu

f32 = jnp.float32
bf16 = jnp.bfloat16

T = 2048
SK = 2048
DM = 576
DH = 128
HKV = 16
FF = 4608
CAP = 8
TT = 256
NSUB = T // TT
CK = 256
NC = SK // CK
EPS = 1e-5
QSCALE = 0.08837890625 * 1.4426950408889634
NT = (((1,), (1,)), ((), ()))

FC = 384
NFC = FF // FC
TR0 = 2
QPOS = 2
OPOS = 1
MROWS = 128
NMX = 4
PIECES = (2, 2, 2, 2)
PSTART = tuple(sum(PIECES[:i]) for i in range(len(PIECES)))
WWAIT = 6
PAD0 = 4


def _rb(x):
    return x.astype(bf16).astype(f32)


def _sigmoid(x):
    return 0.5 * jnp.tanh(0.5 * x) + 0.5


def _silu(x):
    hx = 0.5 * x
    return hx + hx * jnp.tanh(hx)


def _kernel(xt_hbm, k_hbm, v_hbm, wq_hbm, wot_hbm, wr_hbm, wg_hbm, wu_hbm, wdt_hbm,
            out_hbm,
            pad_ref, xt_ref, k_ref, v_ref, wq_ref, wot_ref, xn_ref, gt_ref, acc_ref, out_ref, wdt_ref, wd_ref,
            qc_ref, sc_ref, mc_ref, oc_ref, xs_ref, rs_ref, idx_ref, wg_ref, wu_ref, wr_ref,
            sem_x, sem_r, sem_a, sem_b, sem_moe, sem_out):
    h = pl.program_id(0)

    def cp_x(part):
        cols = pl.ds(PSTART[part] * TT, PIECES[part] * TT)
        return pltpu.make_async_copy(xt_hbm.at[:, cols], xt_ref.at[:, cols], sem_x.at[part])

    def _hcols(hh):
        start = hh * (2 * DH)
        if not isinstance(hh, int):
            start = pl.multiple_of(start, 2 * DH)
        return pl.ds(start, 2 * DH)

    def grp_a(hh):
        first = pl.ds(0, CK)
        return (pltpu.make_async_copy(wq_hbm.at[:, _hcols(hh)], wq_ref.at[hh], sem_a.at[hh]),
                pltpu.make_async_copy(k_hbm.at[hh, first], k_ref.at[hh, first], sem_a.at[hh]))

    def grp_b(hh):
        rest = pl.ds(CK, SK - CK)
        return (pltpu.make_async_copy(k_hbm.at[hh, rest], k_ref.at[hh, rest], sem_b.at[hh]),
                pltpu.make_async_copy(v_hbm.at[hh], v_ref.at[hh], sem_b.at[hh]),
                pltpu.make_async_copy(wot_hbm.at[:, _hcols(hh)], wot_ref.at[hh], sem_b.at[hh]))

    def cp_up():
        return (pltpu.make_async_copy(wg_hbm, wg_ref, sem_moe.at[0]),
                pltpu.make_async_copy(wu_hbm, wu_ref, sem_moe.at[1]))

    def cp_down():
        return [pltpu.make_async_copy(wdt_hbm.at[:, pl.ds(c * FC, FC)], wdt_ref.at[c], sem_moe.at[2])
                for c in range(NFC)]

    def cp_out(t):
        cols = pl.ds(t * TT, TT)
        return pltpu.make_async_copy(out_ref.at[:, cols], out_hbm.at[:, cols], sem_out.at[t])

    def layernorm_tile(t, wr8):
        cols = slice(t * TT, (t + 1) * TT)
        x = xt_ref[:, cols].astype(f32)
        mean = jnp.sum(x, axis=0, keepdims=True) * (1.0 / DM)
        mb = _rb(mean)
        d = x - mb
        dm = mean - mb
        var = jnp.maximum(jnp.sum(d * d, axis=0, keepdims=True) * (1.0 / DM) - dm * dm, 0.0)
        den = _rb(jnp.sqrt(_rb(_rb(var) + EPS)))
        y = _rb(d) * (1.0 / den)
        xb = y.astype(bf16)
        xn = xb.astype(f32)
        xn_ref[cols, :] = xn.T
        gt_ref[:, cols] = _silu(xn)
        return jnp.dot(wr8, xb, preferred_element_type=f32)[0:1]

    def route(r):
        rbits = pltpu.bitcast(_rb(r), jnp.int32) >> 16
        mono = jnp.where(rbits < 0, -(rbits & 0x7FFF), rbits) + 32768
        lane = lax.broadcasted_iota(jnp.int32, (1, T), 1)
        keys = pltpu.bitcast(mono * T + (T - 1 - lane) + (1 << 23), f32)
        for j in range(CAP):
            kv = jnp.max(keys, axis=1, keepdims=True)
            keys = jnp.where(keys == kv, 0.0, keys)
            ki = pltpu.bitcast(kv, jnp.int32) - (1 << 23)
            idx = (T - 1) - (ki[0, 0] & (T - 1))
            idx_ref[j] = idx
            code = (ki >> 11) - 32768
            bits = jnp.where(code < 0, (-code) | 0x8000, code) << 16
            rs_ref[j:j + 1, :] = jnp.broadcast_to(pltpu.bitcast(bits, f32), (1, 128))
            xs_ref[j:j + 1, :] = xn_ref[pl.ds(idx, 1), :]

    def expert():
        xs32 = xs_ref[...]
        xs = xs32.astype(bf16)
        gate = _rb(_silu(_rb(jnp.dot(xs, wg_ref[...], preferred_element_type=f32))))
        up = _rb(jnp.dot(xs, wu_ref[...], preferred_element_type=f32))
        hid = (gate * up).astype(bf16)
        y = _rb(jnp.dot(hid, wd_ref[0:FF, :], preferred_element_type=f32))
        rs = _rb(_sigmoid(rs_ref[:, 0:1]))
        y = _rb(y * rs)
        gnew = _silu(_rb(xs32 + y))
        gnew_t = jnp.concatenate([gnew, jnp.zeros((128 - CAP, DM), f32)], axis=0).T
        lane128 = lax.broadcasted_iota(jnp.int32, (DM, 128), 1)
        gnew_b = gnew_t.astype(bf16)
        row = lax.broadcasted_iota(jnp.int32, (128, 128), 0)
        colk = lax.broadcasted_iota(jnp.int32, (128, 128), 1)
        for j in range(CAP):
            i = idx_ref[j]
            blk = pl.ds(pl.multiple_of((i >> 7) << 7, 128), 128)
            if j < NMX:
                perm = jnp.where(jnp.logical_and(row == j, colk == (i & 127)), 1.0, 0.0).astype(bf16)
                col = jnp.dot(gnew_b, perm, preferred_element_type=f32)
            else:
                col = pltpu.roll(gnew_t, ((i & 127) + (128 - j)) & 127, 1)
            pltpu.store(gt_ref.at[:, blk], col, mask=lane128 == (i & 127))

    def transpose_down():
        active = jnp.logical_and(h >= TR0, h < TR0 + NFC)
        fc = jnp.where(active, h - TR0, NFC)
        rows = pl.ds(pl.multiple_of(fc * FC, FC), FC)
        wd_ref[rows, :] = wdt_ref[fc].astype(f32).T.astype(bf16)

    def qproj(t, w):
        xn = xn_ref[t * TT:(t + 1) * TT, :].astype(bf16)
        q = jnp.dot(xn, w, preferred_element_type=f32) * QSCALE
        q = q.astype(bf16)
        return jnp.concatenate([q[:, :DH], q[:, DH:]], axis=0)

    def qk(q, hh, c):
        return lax.dot_general(q, k_ref[hh, c * CK:(c + 1) * CK, :], NT, preferred_element_type=f32)

    def finalize(lp, o):
        l = jnp.sum(lp, axis=-1, keepdims=True)
        r0 = pl.reciprocal(l, approx=True)
        r = r0 * (2.0 - l * r0)
        o = (o * r).astype(bf16)
        return jnp.concatenate([o[:TT], o[TT:]], axis=1)

    def oproj(o, w):
        return lax.dot_general(w, o, NT, preferred_element_type=f32)

    def combine(cols, s):
        out_ref[:, cols] = (xt_ref[:, cols].astype(f32) + s * gt_ref[:, cols]).astype(bf16)

    def attention_step():
        hn = jnp.minimum(h + 1, HKV - 1)
        hp = jnp.maximum(h - 1, 0)
        q, sc, st, fin = {0: qc_ref[...]}, {(0, 0): sc_ref[...]}, {}, {-1: oc_ref[...]}

        def rowmax(s):
            return jnp.broadcast_to(jnp.max(s, axis=-1, keepdims=True), (s.shape[0], 128))

        def pv(t, c):
            s = sc.pop((t, c))
            vc = v_ref[h, c * CK:(c + 1) * CK, :]
            wide = t == 0
            if t == 0 and c == 0:
                mc = jnp.concatenate([mc_ref[...], rowmax(s[MROWS:])], axis=0)
            elif wide:
                mc = rowmax(s)
            else:
                mc = jnp.max(s, axis=-1, keepdims=True)

            def probs(m):
                if wide:
                    return jnp.concatenate([jnp.exp2(s[:, j * 128:(j + 1) * 128] - m)
                                            for j in range(CK // 128)], axis=1)
                return jnp.exp2(s - m)

            if c == 0:
                m = mc
                p = probs(m)
                lp = p[:, 0:128]
                for j in range(1, CK // 128):
                    lp = lp + p[:, j * 128:(j + 1) * 128]
                o = jnp.dot(p.astype(bf16), vc, preferred_element_type=f32)
            else:
                m0, lp0, o0 = st[t]
                m = jnp.maximum(m0, mc)
                a = jnp.exp2(m0 - m)
                p = probs(m)
                pvp = jnp.dot(p.astype(bf16), vc, preferred_element_type=f32)
                lp = lp0 * a
                for j in range(CK // 128):
                    lp = lp + p[:, j * 128:(j + 1) * 128]
                o = pvp + o0 * a
            st[t] = (m, lp, o)
            if c == NC - 1:
                del st[t]
                if t == NSUB - 1:
                    oc_ref[...] = finalize(lp, o)
                else:
                    fin[t] = finalize(lp, o)

        items = [(t, c) for t in range(NSUB) for c in range(NC)]
        n = len(items)
        for i in range(n):
            if i == 0:
                transpose_down()
            if 8 <= i < 8 + NFC:
                @pl.when(h == 0)
                def _():
                    cp_down()[i - 8].start()
            t1, c1 = items[i + 1] if i + 1 < n else (NSUB, 0)
            if t1 < NSUB:
                sc[(t1, c1)] = qk(q[t1], h, c1)
            else:
                s_next = qk(q[t1], hn, 0)
                sc_ref[...] = s_next
                mc_ref[...] = rowmax(s_next[0:MROWS])
            t, c = items[i]
            pv(t, c)
            if c == OPOS:
                tp = (t - 1) % NSUB
                w = wot_ref[hp] if t == 0 else wot_ref[h]
                cols = slice(tp * TT, (tp + 1) * TT)
                s_new = acc_ref[:, cols] + oproj(fin.pop(t - 1), w)
                acc_ref[:, cols] = s_new
                if t > 0:
                    combine(cols, s_new)

                    @pl.when(h == HKV - 1)
                    def _():
                        cp_out(tp).start()
            if c1 == QPOS:
                tq = t1 + 1
                if tq < NSUB:
                    q[tq] = qproj(tq, wq_ref[h])
                else:
                    q[tq] = qproj(0, wq_ref[hn])
                    qc_ref[...] = q[tq]

    @pl.when(h == 0)
    def _prologue():
        cp_r = pltpu.make_async_copy(wr_hbm, wr_ref, sem_r)
        k_rest, v0, wo0 = grp_b(0)
        stages = {0: [cp_x(2)] + list(grp_a(0)), 1: [cp_x(3), v0], 2: [k_rest, wo0], 3: list(grp_a(1))}
        for c in (cp_x(0), cp_r, cp_x(1)):
            c.start()
        acc_ref[...] = jnp.zeros((DM, T), f32)
        oc_ref[...] = jnp.zeros((TT, 2 * DH), bf16)
        pad_ref[0:8, :] = jnp.zeros((8, 128), f32)
        rparts = []
        for t in range(NSUB):
            if t in PSTART:
                cp_x(PSTART.index(t)).wait()
                if t == 0:
                    cp_r.wait()
                    wr8 = jnp.broadcast_to(wr_ref[...].reshape(1, DM), (8, DM))
                for c in stages[PSTART.index(t)]:
                    c.start()
            if t == WWAIT:
                for c in grp_a(0):
                    c.wait()
            rparts.append(layernorm_tile(t, wr8))
        route(jnp.concatenate(rparts, axis=1))
        q0 = qproj(0, wq_ref[0])
        qc_ref[...] = q0
        s0 = qk(q0, 0, 0)
        sc_ref[...] = s0
        mc_ref[...] = jnp.broadcast_to(jnp.max(s0[0:MROWS], axis=-1, keepdims=True), (MROWS, 128))

    for c in grp_b(h):
        c.wait()

    @pl.when(h + 1 < HKV)
    def _():
        for c in grp_a(h + 1):
            c.wait()
        for c in grp_b(h + 1):
            c.start()

    @pl.when(h + 2 < HKV)
    def _():
        for c in grp_a(h + 2):
            c.start()

    @pl.when(h == TR0)
    def _():
        all_chunks = wdt_ref.at[pl.ds(0, NFC)]
        pltpu.make_async_copy(all_chunks, all_chunks, sem_moe.at[2]).wait()
        for c in cp_up():
            c.start()

    @pl.when(h == TR0 + NFC)
    def _():
        for c in cp_up():
            c.wait()
        expert()

    attention_step()

    @pl.when(h == HKV - 1)
    def _epilogue():
        tl = NSUB - 1
        cols = slice(tl * TT, T)
        combine(cols, acc_ref[:, cols] + oproj(oc_ref[...], wot_ref[HKV - 1]))
        cp_out(tl).start()
        for t in range(NSUB):
            cp_out(t).wait()


@jax.jit
def pallas_recurrent_scan__gqa_block_cached__moe_arch_mod__prompt_kernel(
    A_x: jax.Array,
    A_k_cache: jax.Array,
    A_v_cache: jax.Array,
    A_wq: jax.Array,
    A_wo: jax.Array,
    B_x: jax.Array,
    B_w_r: jax.Array,
    B_w_gate: jax.Array,
    B_w_up: jax.Array,
    B_w_down: jax.Array,
):
    del B_x
    xt = A_x.reshape(T, DM).T
    k = A_k_cache.reshape(HKV, SK, DH)
    v = A_v_cache.reshape(HKV, SK, DH)
    wot = A_wo.T
    wdt = B_w_down.T
    hbm = pl.BlockSpec(memory_space=pl.ANY)
    dma = pltpu.SemaphoreType.DMA
    out_t = pl.pallas_call(
        _kernel,
        out_shape=jax.ShapeDtypeStruct((DM, T), bf16),
        grid=(HKV,),
        in_specs=[hbm] * 9,
        out_specs=hbm,
        scratch_shapes=[
            pltpu.VMEM((8 * PAD0, 128), f32),
            pltpu.VMEM((DM, T), bf16),
            pltpu.VMEM((HKV, SK, DH), bf16),
            pltpu.VMEM((HKV, SK, DH), bf16),
            pltpu.VMEM((HKV, DM, 2 * DH), bf16),
            pltpu.VMEM((HKV, DM, 2 * DH), bf16),
            pltpu.VMEM((T, DM), f32),
            pltpu.VMEM((DM, T), f32),
            pltpu.VMEM((DM, T), f32),
            pltpu.VMEM((DM, T), bf16),
            pltpu.VMEM((NFC + 1, DM, FC), bf16),
            pltpu.VMEM((FF + FC, DM), bf16),
            pltpu.VMEM((2 * TT, DH), bf16),
            pltpu.VMEM((2 * TT, CK), f32),
            pltpu.VMEM((MROWS, 128), f32),
            pltpu.VMEM((TT, 2 * DH), bf16),
            pltpu.VMEM((CAP, DM), f32),
            pltpu.VMEM((CAP, 128), f32),
            pltpu.SMEM((CAP,), jnp.int32),
            pltpu.VMEM((DM, FF), bf16),
            pltpu.VMEM((DM, FF), bf16),
            pltpu.VMEM((DM,), bf16),
            dma((len(PIECES),)), dma(()), dma((HKV,)), dma((HKV,)), dma((3,)), dma((NSUB,)),
        ],
        compiler_params=pltpu.CompilerParams(
            dimension_semantics=("arbitrary",),
            disable_bounds_checks=True,
            vmem_limit_bytes=120 * 1024 * 1024,
        ),
    )(xt, k, v, A_wq, wot, B_w_r, B_w_gate, B_w_up, wdt)
    return out_t.T.reshape(1, T, DM)
```

```python
import jax
import jax.numpy as jnp
from jax import lax
import jax.experimental.pallas as pl
import jax.experimental.pallas.tpu as pltpu

f32 = jnp.float32
bf16 = jnp.bfloat16

T = 2048
SK = 2048
DM = 576
DH = 128
HKV = 16
FF = 4608
CAP = 8
TT = 256
NSUB = T // TT
CK = 256
NC = SK // CK
EPS = 1e-5
QSCALE = 0.08837890625 * 1.4426950408889634
NT = (((1,), (1,)), ((), ()))

FC = 384
NFC = FF // FC
TR0 = 2
QPOS = 2
OPOS = 1
MROWS = 128
NLAST = 3
NMX = 4
PIECES = (2, 2, 2, 2)
PSTART = tuple(sum(PIECES[:i]) for i in range(len(PIECES)))
WWAIT = 6
PAD0 = 4


def _rb(x):
    return x.astype(bf16).astype(f32)


def _sigmoid(x):
    return 0.5 * jnp.tanh(0.5 * x) + 0.5


def _silu(x):
    hx = 0.5 * x
    return hx + hx * jnp.tanh(hx)


def _kernel(xt_hbm, k_hbm, v_hbm, wq_hbm, wot_hbm, wr_hbm, wg_hbm, wu_hbm, wdt_hbm,
            out_hbm,
            pad_ref, xt_ref, k_ref, v_ref, wq_ref, wot_ref, xn_ref, gt_ref, acc_ref, out_ref, wdt_ref, wd_ref,
            qc_ref, sc_ref, mc_ref, oc_ref, xs_ref, rs_ref, idx_ref, wg_ref, wu_ref, wr_ref,
            sem_x, sem_r, sem_a, sem_b, sem_moe, sem_out):
    h = pl.program_id(0)

    def cp_x(part):
        cols = pl.ds(PSTART[part] * TT, PIECES[part] * TT)
        return pltpu.make_async_copy(xt_hbm.at[:, cols], xt_ref.at[:, cols], sem_x.at[part])

    def _hcols(hh):
        start = hh * (2 * DH)
        if not isinstance(hh, int):
            start = pl.multiple_of(start, 2 * DH)
        return pl.ds(start, 2 * DH)

    def grp_a(hh):
        first = pl.ds(0, CK)
        return (pltpu.make_async_copy(wq_hbm.at[:, _hcols(hh)], wq_ref.at[hh], sem_a.at[hh]),
                pltpu.make_async_copy(k_hbm.at[hh, first], k_ref.at[hh, first], sem_a.at[hh]))

    def grp_b(hh):
        rest = pl.ds(CK, SK - CK)
        return (pltpu.make_async_copy(k_hbm.at[hh, rest], k_ref.at[hh, rest], sem_b.at[hh]),
                pltpu.make_async_copy(v_hbm.at[hh], v_ref.at[hh], sem_b.at[hh]),
                pltpu.make_async_copy(wot_hbm.at[:, _hcols(hh)], wot_ref.at[hh], sem_b.at[hh]))

    def cp_up():
        return (pltpu.make_async_copy(wg_hbm, wg_ref, sem_moe.at[0]),
                pltpu.make_async_copy(wu_hbm, wu_ref, sem_moe.at[1]))

    def cp_down():
        return [pltpu.make_async_copy(wdt_hbm.at[:, pl.ds(c * FC, FC)], wdt_ref.at[c], sem_moe.at[2])
                for c in range(NFC)]

    def cp_out(t):
        cols = pl.ds(t * TT, TT)
        return pltpu.make_async_copy(out_ref.at[:, cols], out_hbm.at[:, cols], sem_out.at[t])

    def layernorm_tile(t, wr8):
        cols = slice(t * TT, (t + 1) * TT)
        x = xt_ref[:, cols].astype(f32)
        mean = jnp.sum(x, axis=0, keepdims=True) * (1.0 / DM)
        mb = _rb(mean)
        d = x - mb
        dm = mean - mb
        var = jnp.maximum(jnp.sum(d * d, axis=0, keepdims=True) * (1.0 / DM) - dm * dm, 0.0)
        den = _rb(jnp.sqrt(_rb(_rb(var) + EPS)))
        y = _rb(d) * (1.0 / den)
        xb = y.astype(bf16)
        xn = xb.astype(f32)
        xn_ref[cols, :] = xn.T
        gt_ref[:, cols] = _silu(xn)
        return jnp.dot(wr8, xb, preferred_element_type=f32)[0:1]

    def route(r):
        rbits = pltpu.bitcast(_rb(r), jnp.int32) >> 16
        mono = jnp.where(rbits < 0, -(rbits & 0x7FFF), rbits) + 32768
        lane = lax.broadcasted_iota(jnp.int32, (1, T), 1)
        keys = pltpu.bitcast(mono * T + (T - 1 - lane) + (1 << 23), f32)
        for j in range(CAP):
            kv = jnp.max(keys, axis=1, keepdims=True)
            keys = jnp.where(keys == kv, 0.0, keys)
            ki = pltpu.bitcast(kv, jnp.int32) - (1 << 23)
            idx = (T - 1) - (ki[0, 0] & (T - 1))
            idx_ref[j] = idx
            code = (ki >> 11) - 32768
            bits = jnp.where(code < 0, (-code) | 0x8000, code) << 16
            rs_ref[j:j + 1, :] = jnp.broadcast_to(pltpu.bitcast(bits, f32), (1, 128))
            xs_ref[j:j + 1, :] = xn_ref[pl.ds(idx, 1), :]

    def expert():
        xs32 = xs_ref[...]
        xs = xs32.astype(bf16)
        gate = _rb(_silu(_rb(jnp.dot(xs, wg_ref[...], preferred_element_type=f32))))
        up = _rb(jnp.dot(xs, wu_ref[...], preferred_element_type=f32))
        hid = (gate * up).astype(bf16)
        y = _rb(jnp.dot(hid, wd_ref[0:FF, :], preferred_element_type=f32))
        rs = _rb(_sigmoid(rs_ref[:, 0:1]))
        y = _rb(y * rs)
        gnew = _silu(_rb(xs32 + y))
        gnew_t = jnp.concatenate([gnew, jnp.zeros((128 - CAP, DM), f32)], axis=0).T
        lane128 = lax.broadcasted_iota(jnp.int32, (DM, 128), 1)
        gnew_b = gnew_t.astype(bf16)
        row = lax.broadcasted_iota(jnp.int32, (128, 128), 0)
        colk = lax.broadcasted_iota(jnp.int32, (128, 128), 1)
        for j in range(CAP):
            i = idx_ref[j]
            blk = pl.ds(pl.multiple_of((i >> 7) << 7, 128), 128)
            if j < NMX:
                perm = jnp.where(jnp.logical_and(row == j, colk == (i & 127)), 1.0, 0.0).astype(bf16)
                col = jnp.dot(gnew_b, perm, preferred_element_type=f32)
            else:
                col = pltpu.roll(gnew_t, ((i & 127) + (128 - j)) & 127, 1)
            pltpu.store(gt_ref.at[:, blk], col, mask=lane128 == (i & 127))

    def transpose_down():
        active = jnp.logical_and(h >= TR0, h < TR0 + NFC)
        fc = jnp.where(active, h - TR0, NFC)
        rows = pl.ds(pl.multiple_of(fc * FC, FC), FC)
        wd_ref[rows, :] = wdt_ref[fc].astype(f32).T.astype(bf16)

    def qproj(t, w):
        xn = xn_ref[t * TT:(t + 1) * TT, :].astype(bf16)
        q = jnp.dot(xn, w, preferred_element_type=f32) * QSCALE
        q = q.astype(bf16)
        return jnp.concatenate([q[:, :DH], q[:, DH:]], axis=0)

    def qk(q, hh, c):
        return lax.dot_general(q, k_ref[hh, c * CK:(c + 1) * CK, :], NT, preferred_element_type=f32)

    def finalize(lp, o):
        l = jnp.sum(lp, axis=-1, keepdims=True)
        r0 = pl.reciprocal(l, approx=True)
        r = r0 * (2.0 - l * r0)
        o = (o * r).astype(bf16)
        return jnp.concatenate([o[:TT], o[TT:]], axis=1)

    def oproj(o, w):
        return lax.dot_general(w, o, NT, preferred_element_type=f32)

    def combine(cols, s):
        out_ref[:, cols] = (xt_ref[:, cols].astype(f32) + s * gt_ref[:, cols]).astype(bf16)

    def attention_step():
        hn = jnp.minimum(h + 1, HKV - 1)
        hp = jnp.maximum(h - 1, 0)
        q, sc, st, fin = {0: qc_ref[...]}, {(0, 0): sc_ref[...]}, {}, {-1: oc_ref[...]}

        def rowmax(s):
            return jnp.broadcast_to(jnp.max(s, axis=-1, keepdims=True), (s.shape[0], 128))

        def pv(t, c):
            s = sc.pop((t, c))
            vc = v_ref[h, c * CK:(c + 1) * CK, :]
            wide = t == 0
            if t == 0 and c == 0:
                mc = jnp.concatenate([mc_ref[...], rowmax(s[MROWS:])], axis=0)
            elif wide:
                mc = rowmax(s)
            else:
                mc = jnp.max(s, axis=-1, keepdims=True)

            def probs(m):
                if wide:
                    return jnp.concatenate([jnp.exp2(s[:, j * 128:(j + 1) * 128] - m)
                                            for j in range(CK // 128)], axis=1)
                return jnp.exp2(s - m)

            if c == 0:
                m = mc
                p = probs(m)
                lp = p[:, 0:128]
                for j in range(1, CK // 128):
                    lp = lp + p[:, j * 128:(j + 1) * 128]
                o = jnp.dot(p.astype(bf16), vc, preferred_element_type=f32)
            else:
                m0, lp0, o0 = st[t]
                m = jnp.maximum(m0, mc)
                a = jnp.exp2(m0 - m)
                p = probs(m)
                pvp = jnp.dot(p.astype(bf16), vc, preferred_element_type=f32)
                lp = lp0 * a
                for j in range(CK // 128):
                    lp = lp + p[:, j * 128:(j + 1) * 128]
                o = pvp + o0 * a
            st[t] = (m, lp, o)
            if c == NC - 1:
                del st[t]
                if t == NSUB - 1:
                    oc_ref[...] = finalize(lp, o)
                else:
                    fin[t] = finalize(lp, o)

        items = [(t, c) for t in range(NSUB) for c in range(NC)]
        n = len(items)
        for i in range(n):
            if i == 0:
                transpose_down()
            if 8 <= i < 8 + NFC:
                @pl.when(h == 0)
                def _():
                    cp_down()[i - 8].start()
            t1, c1 = items[i + 1] if i + 1 < n else (NSUB, 0)
            if t1 < NSUB:
                sc[(t1, c1)] = qk(q[t1], h, c1)
            else:
                s_next = qk(q[t1], hn, 0)
                sc_ref[...] = s_next
                mc_ref[...] = rowmax(s_next[0:MROWS])
            t, c = items[i]
            pv(t, c)
            if c == OPOS:
                tp = (t - 1) % NSUB
                w = wot_ref[hp] if t == 0 else wot_ref[h]
                cols = slice(tp * TT, (tp + 1) * TT)
                s_new = acc_ref[:, cols] + oproj(fin.pop(t - 1), w)
                acc_ref[:, cols] = s_new
                if t > 0:
                    combine(cols, s_new)

                    @pl.when(h == HKV - 1)
                    def _():
                        cp_out(tp).start()
            if c1 == QPOS:
                tq = t1 + 1
                if tq < NSUB:
                    q[tq] = qproj(tq, wq_ref[h])
                else:
                    q[tq] = qproj(0, wq_ref[hn])
                    qc_ref[...] = q[tq]

    @pl.when(h == 0)
    def _prologue():
        cp_r = pltpu.make_async_copy(wr_hbm, wr_ref, sem_r)
        k_rest, v0, wo0 = grp_b(0)
        stages = {0: [cp_x(2)] + list(grp_a(0)), 1: [cp_x(3), v0], 2: [k_rest, wo0], 3: list(grp_a(1))}
        for c in (cp_x(0), cp_r, cp_x(1)):
            c.start()
        acc_ref[...] = jnp.zeros((DM, T), f32)
        oc_ref[...] = jnp.zeros((TT, 2 * DH), bf16)
        pad_ref[0:8, :] = jnp.zeros((8, 128), f32)
        rparts = []
        for t in range(NSUB):
            if t in PSTART:
                cp_x(PSTART.index(t)).wait()
                if t == 0:
                    cp_r.wait()
                    wr8 = jnp.broadcast_to(wr_ref[...].reshape(1, DM), (8, DM))
                for c in stages[PSTART.index(t)]:
                    c.start()
            if t == WWAIT:
                for c in grp_a(0):
                    c.wait()
            rparts.append(layernorm_tile(t, wr8))
        route(jnp.concatenate(rparts, axis=1))
        q0 = qproj(0, wq_ref[0])
        qc_ref[...] = q0
        s0 = qk(q0, 0, 0)
        sc_ref[...] = s0
        mc_ref[...] = jnp.broadcast_to(jnp.max(s0[0:MROWS], axis=-1, keepdims=True), (MROWS, 128))

    for c in grp_b(h):
        c.wait()

    @pl.when(h + 1 < HKV)
    def _():
        for c in grp_a(h + 1):
            c.wait()
        for c in grp_b(h + 1):
            c.start()

    @pl.when(h + 2 < HKV)
    def _():
        for c in grp_a(h + 2):
            c.start()

    @pl.when(h == TR0)
    def _():
        all_chunks = wdt_ref.at[pl.ds(0, NFC)]
        pltpu.make_async_copy(all_chunks, all_chunks, sem_moe.at[2]).wait()
        for c in cp_up():
            c.start()

    @pl.when(h == TR0 + NFC)
    def _():
        for c in cp_up():
            c.wait()
        expert()

    attention_step()

    @pl.when(h == HKV - 1)
    def _epilogue():
        tl = NSUB - 1
        cols = slice(tl * TT, T)
        o_last = oc_ref[...]
        tail = []
        for b in range(NLAST):
            rows = slice(b * (DM // NLAST), (b + 1) * (DM // NLAST))
            s = acc_ref[rows, cols] + oproj(o_last, wot_ref[HKV - 1, rows, :])
            out_ref[rows, cols] = (xt_ref[rows, cols].astype(f32) + s * gt_ref[rows, cols]).astype(bf16)
            dst = (pl.ds(rows.start, DM // NLAST), pl.ds(tl * TT, TT))
            tail.append(pltpu.make_async_copy(out_ref.at[dst], out_hbm.at[dst], sem_out.at[tl + b]))
            tail[-1].start()
        for t in range(tl):
            cp_out(t).wait()
        for c in tail:
            c.wait()


@jax.jit
def pallas_recurrent_scan__gqa_block_cached__moe_arch_mod__prompt_kernel(
    A_x: jax.Array,
    A_k_cache: jax.Array,
    A_v_cache: jax.Array,
    A_wq: jax.Array,
    A_wo: jax.Array,
    B_x: jax.Array,
    B_w_r: jax.Array,
    B_w_gate: jax.Array,
    B_w_up: jax.Array,
    B_w_down: jax.Array,
):
    del B_x
    xt = A_x.reshape(T, DM).T
    k = A_k_cache.reshape(HKV, SK, DH)
    v = A_v_cache.reshape(HKV, SK, DH)
    wot = A_wo.T
    wdt = B_w_down.T
    hbm = pl.BlockSpec(memory_space=pl.ANY)
    dma = pltpu.SemaphoreType.DMA
    out_t = pl.pallas_call(
        _kernel,
        out_shape=jax.ShapeDtypeStruct((DM, T), bf16),
        grid=(HKV,),
        in_specs=[hbm] * 9,
        out_specs=hbm,
        scratch_shapes=[
            pltpu.VMEM((8 * PAD0, 128), f32),
            pltpu.VMEM((DM, T), bf16),
            pltpu.VMEM((HKV, SK, DH), bf16),
            pltpu.VMEM((HKV, SK, DH), bf16),
            pltpu.VMEM((HKV, DM, 2 * DH), bf16),
            pltpu.VMEM((HKV, DM, 2 * DH), bf16),
            pltpu.VMEM((T, DM), f32),
            pltpu.VMEM((DM, T), f32),
            pltpu.VMEM((DM, T), f32),
            pltpu.VMEM((DM, T), bf16),
            pltpu.VMEM((NFC + 1, DM, FC), bf16),
            pltpu.VMEM((FF + FC, DM), bf16),
            pltpu.VMEM((2 * TT, DH), bf16),
            pltpu.VMEM((2 * TT, CK), f32),
            pltpu.VMEM((MROWS, 128), f32),
            pltpu.VMEM((TT, 2 * DH), bf16),
            pltpu.VMEM((CAP, DM), f32),
            pltpu.VMEM((CAP, 128), f32),
            pltpu.SMEM((CAP,), jnp.int32),
            pltpu.VMEM((DM, FF), bf16),
            pltpu.VMEM((DM, FF), bf16),
            pltpu.VMEM((DM,), bf16),
            dma((len(PIECES),)), dma(()), dma((HKV,)), dma((HKV,)), dma((3,)), dma((NSUB - 1 + NLAST,)),
        ],
        compiler_params=pltpu.CompilerParams(
            dimension_semantics=("arbitrary",),
            disable_bounds_checks=True,
            vmem_limit_bytes=120 * 1024 * 1024,
        ),
    )(xt, k, v, A_wq, wot, B_w_r, B_w_gate, B_w_up, wdt)
    return out_t.T.reshape(1, T, DM)
```

```python
import jax
import jax.numpy as jnp
from jax import lax
import jax.experimental.pallas as pl
import jax.experimental.pallas.tpu as pltpu

f32 = jnp.float32
bf16 = jnp.bfloat16

T = 2048
SK = 2048
DM = 576
DH = 128
HKV = 16
FF = 4608
CAP = 8
TT = 256
NSUB = T // TT
CK = 256
NC = SK // CK
EPS = 1e-5
QSCALE = 0.08837890625 * 1.4426950408889634
NT = (((1,), (1,)), ((), ()))

FC = 384
NFC = FF // FC
TR0 = 2
QPOS = 2
OPOS = 1
MROWS = 128
NLAST = 3
NMX = 4
PIECES = (2, 2, 2, 2)
PSTART = tuple(sum(PIECES[:i]) for i in range(len(PIECES)))
WWAIT = 6
PAD0 = 4


def _rb(x):
    return x.astype(bf16).astype(f32)


def _sigmoid(x):
    return 0.5 * jnp.tanh(0.5 * x) + 0.5


def _silu(x):
    hx = 0.5 * x
    return hx + hx * jnp.tanh(hx)


def _kernel(xt_hbm, k_hbm, v_hbm, wq_hbm, wot_hbm, wr_hbm, wg_hbm, wu_hbm, wdt_hbm,
            out_hbm,
            pad_ref, xt_ref, k_ref, v_ref, wq_ref, wot_ref, xn_ref, gt_ref, acc_ref, out_ref, wdt_ref, wd_ref,
            qc_ref, sc_ref, mc_ref, oc_ref, xs_ref, rs_ref, idx_ref, wg_ref, wu_ref, wr_ref,
            sem_x, sem_r, sem_a, sem_b, sem_moe, sem_out):
    h = pl.program_id(0)

    def cp_x(part):
        cols = pl.ds(PSTART[part] * TT, PIECES[part] * TT)
        return pltpu.make_async_copy(xt_hbm.at[:, cols], xt_ref.at[:, cols], sem_x.at[part])

    def _hcols(hh):
        start = hh * (2 * DH)
        if not isinstance(hh, int):
            start = pl.multiple_of(start, 2 * DH)
        return pl.ds(start, 2 * DH)

    def grp_a(hh):
        first = pl.ds(0, CK)
        return (pltpu.make_async_copy(wq_hbm.at[:, _hcols(hh)], wq_ref.at[hh], sem_a.at[hh]),
                pltpu.make_async_copy(k_hbm.at[hh, first], k_ref.at[hh, first], sem_a.at[hh]))

    def grp_b(hh):
        rest = pl.ds(CK, SK - CK)
        return (pltpu.make_async_copy(k_hbm.at[hh, rest], k_ref.at[hh, rest], sem_b.at[hh]),
                pltpu.make_async_copy(v_hbm.at[hh], v_ref.at[hh], sem_b.at[hh]),
                pltpu.make_async_copy(wot_hbm.at[:, _hcols(hh)], wot_ref.at[hh], sem_b.at[hh]))

    def cp_up():
        return (pltpu.make_async_copy(wg_hbm, wg_ref, sem_moe.at[0]),
                pltpu.make_async_copy(wu_hbm, wu_ref, sem_moe.at[1]))

    def cp_down(c):
        return pltpu.make_async_copy(wdt_hbm.at[:, pl.ds(c * FC, FC)], wdt_ref.at[c], sem_moe.at[2])

    def cp_out(t):
        cols = pl.ds(t * TT, TT)
        return pltpu.make_async_copy(out_ref.at[:, cols], out_hbm.at[:, cols], sem_out.at[t])

    def layernorm_tile(t, wr8):
        cols = slice(t * TT, (t + 1) * TT)
        x = xt_ref[:, cols].astype(f32)
        mean = jnp.sum(x, axis=0, keepdims=True) * (1.0 / DM)
        mb = _rb(mean)
        d = x - mb
        dm = mean - mb
        var = jnp.maximum(jnp.sum(d * d, axis=0, keepdims=True) * (1.0 / DM) - dm * dm, 0.0)
        den = _rb(jnp.sqrt(_rb(_rb(var) + EPS)))
        y = _rb(d) * (1.0 / den)
        xb = y.astype(bf16)
        xn = xb.astype(f32)
        xn_ref[cols, :] = xn.T
        gt_ref[:, cols] = _silu(xn)
        return jnp.dot(wr8, xb, preferred_element_type=f32)[0:1]

    def route(r):
        rbits = pltpu.bitcast(_rb(r), jnp.int32) >> 16
        mono = jnp.where(rbits < 0, -(rbits & 0x7FFF), rbits) + 32768
        lane = lax.broadcasted_iota(jnp.int32, (1, T), 1)
        keys = pltpu.bitcast(mono * T + (T - 1 - lane) + (1 << 23), f32)
        for j in range(CAP):
            kv = jnp.max(keys, axis=1, keepdims=True)
            keys = jnp.where(keys == kv, 0.0, keys)
            ki = pltpu.bitcast(kv, jnp.int32) - (1 << 23)
            idx = (T - 1) - (ki[0, 0] & (T - 1))
            idx_ref[j] = idx
            code = (ki >> 11) - 32768
            bits = jnp.where(code < 0, (-code) | 0x8000, code) << 16
            rs_ref[j:j + 1, :] = jnp.broadcast_to(pltpu.bitcast(bits, f32), (1, 128))
            xs_ref[j:j + 1, :] = xn_ref[pl.ds(idx, 1), :]

    def expert():
        xs32 = xs_ref[...]
        xs = xs32.astype(bf16)
        gate = _rb(_silu(_rb(jnp.dot(xs, wg_ref[...], preferred_element_type=f32))))
        up = _rb(jnp.dot(xs, wu_ref[...], preferred_element_type=f32))
        hid = (gate * up).astype(bf16)
        y = _rb(jnp.dot(hid, wd_ref[0:FF, :], preferred_element_type=f32))
        rs = _rb(_sigmoid(rs_ref[:, 0:1]))
        y = _rb(y * rs)
        gnew = _silu(_rb(xs32 + y))
        gnew_t = jnp.concatenate([gnew, jnp.zeros((128 - CAP, DM), f32)], axis=0).T
        lane128 = lax.broadcasted_iota(jnp.int32, (DM, 128), 1)
        gnew_b = gnew_t.astype(bf16)
        row = lax.broadcasted_iota(jnp.int32, (128, 128), 0)
        colk = lax.broadcasted_iota(jnp.int32, (128, 128), 1)
        for j in range(CAP):
            i = idx_ref[j]
            blk = pl.ds(pl.multiple_of((i >> 7) << 7, 128), 128)
            if j < NMX:
                perm = jnp.where(jnp.logical_and(row == j, colk == (i & 127)), 1.0, 0.0).astype(bf16)
                col = jnp.dot(gnew_b, perm, preferred_element_type=f32)
            else:
                col = pltpu.roll(gnew_t, ((i & 127) + (128 - j)) & 127, 1)
            pltpu.store(gt_ref.at[:, blk], col, mask=lane128 == (i & 127))

    def transpose_down():
        active = jnp.logical_and(h >= TR0, h < TR0 + NFC)
        fc = jnp.where(active, h - TR0, NFC)
        rows = pl.ds(pl.multiple_of(fc * FC, FC), FC)
        wd_ref[rows, :] = wdt_ref[fc].astype(f32).T.astype(bf16)

    def qproj(t, w):
        xn = xn_ref[t * TT:(t + 1) * TT, :].astype(bf16)
        q = jnp.dot(xn, w, preferred_element_type=f32) * QSCALE
        q = q.astype(bf16)
        return jnp.concatenate([q[:, :DH], q[:, DH:]], axis=0)

    def qk(q, hh, c):
        return lax.dot_general(q, k_ref[hh, c * CK:(c + 1) * CK, :], NT, preferred_element_type=f32)

    def finalize(lp, o):
        l = jnp.sum(lp, axis=-1, keepdims=True)
        r0 = pl.reciprocal(l, approx=True)
        r = r0 * (2.0 - l * r0)
        o = (o * r).astype(bf16)
        return jnp.concatenate([o[:TT], o[TT:]], axis=1)

    def oproj(o, w):
        return lax.dot_general(w, o, NT, preferred_element_type=f32)

    def combine(cols, s):
        out_ref[:, cols] = (xt_ref[:, cols].astype(f32) + s * gt_ref[:, cols]).astype(bf16)

    def attention_step():
        hn = jnp.minimum(h + 1, HKV - 1)
        hp = jnp.maximum(h - 1, 0)
        q, sc, st, fin = {0: qc_ref[...]}, {(0, 0): sc_ref[...]}, {}, {-1: oc_ref[...]}

        def rowmax(s):
            return jnp.broadcast_to(jnp.max(s, axis=-1, keepdims=True), (s.shape[0], 128))

        def pv(t, c):
            s = sc.pop((t, c))
            vc = v_ref[h, c * CK:(c + 1) * CK, :]
            wide = t == 0
            if t == 0 and c == 0:
                mc = jnp.concatenate([mc_ref[...], rowmax(s[MROWS:])], axis=0)
            elif wide:
                mc = rowmax(s)
            else:
                mc = jnp.max(s, axis=-1, keepdims=True)

            def probs(m):
                if wide:
                    return jnp.concatenate([jnp.exp2(s[:, j * 128:(j + 1) * 128] - m)
                                            for j in range(CK // 128)], axis=1)
                return jnp.exp2(s - m)

            if c == 0:
                m = mc
                p = probs(m)
                lp = p[:, 0:128]
                for j in range(1, CK // 128):
                    lp = lp + p[:, j * 128:(j + 1) * 128]
                o = jnp.dot(p.astype(bf16), vc, preferred_element_type=f32)
            else:
                m0, lp0, o0 = st[t]
                m = jnp.maximum(m0, mc)
                a = jnp.exp2(m0 - m)
                p = probs(m)
                pvp = jnp.dot(p.astype(bf16), vc, preferred_element_type=f32)
                lp = lp0 * a
                for j in range(CK // 128):
                    lp = lp + p[:, j * 128:(j + 1) * 128]
                o = pvp + o0 * a
            st[t] = (m, lp, o)
            if c == NC - 1:
                del st[t]
                if t == NSUB - 1:
                    oc_ref[...] = finalize(lp, o)
                else:
                    fin[t] = finalize(lp, o)

        items = [(t, c) for t in range(NSUB) for c in range(NC)]
        n = len(items)
        for i in range(n):
            if i == 0:
                transpose_down()
            if 8 <= i < 8 + NFC:
                @pl.when(h == 0)
                def _():
                    cp_down(i - 8).start()
            t1, c1 = items[i + 1] if i + 1 < n else (NSUB, 0)
            if t1 < NSUB:
                sc[(t1, c1)] = qk(q[t1], h, c1)
            else:
                s_next = qk(q[t1], hn, 0)
                sc_ref[...] = s_next
                mc_ref[...] = rowmax(s_next[0:MROWS])
            t, c = items[i]
            pv(t, c)
            if c == OPOS:
                tp = (t - 1) % NSUB
                w = wot_ref[hp] if t == 0 else wot_ref[h]
                cols = slice(tp * TT, (tp + 1) * TT)
                s_new = acc_ref[:, cols] + oproj(fin.pop(t - 1), w)
                acc_ref[:, cols] = s_new
                if t > 0:
                    combine(cols, s_new)

                    @pl.when(h == HKV - 1)
                    def _():
                        cp_out(tp).start()
            if c1 == QPOS:
                tq = t1 + 1
                if tq < NSUB:
                    q[tq] = qproj(tq, wq_ref[h])
                else:
                    q[tq] = qproj(0, wq_ref[hn])
                    qc_ref[...] = q[tq]

    @pl.when(h == 0)
    def _prologue():
        cp_r = pltpu.make_async_copy(wr_hbm, wr_ref, sem_r)
        k_rest, v0, wo0 = grp_b(0)
        stages = {0: [cp_x(2)] + list(grp_a(0)), 1: [cp_x(3), v0], 2: [k_rest, wo0], 3: list(grp_a(1))}
        for c in (cp_x(0), cp_r, cp_x(1)):
            c.start()
        acc_ref[...] = jnp.zeros((DM, T), f32)
        oc_ref[...] = jnp.zeros((TT, 2 * DH), bf16)
        pad_ref[0:8, :] = jnp.zeros((8, 128), f32)
        rparts = []
        for t in range(NSUB):
            if t in PSTART:
                cp_x(PSTART.index(t)).wait()
                if t == 0:
                    cp_r.wait()
                    wr8 = jnp.broadcast_to(wr_ref[...].reshape(1, DM), (8, DM))
                for c in stages[PSTART.index(t)]:
                    c.start()
            if t == WWAIT:
                for c in grp_a(0):
                    c.wait()
            rparts.append(layernorm_tile(t, wr8))
        route(jnp.concatenate(rparts, axis=1))
        q0 = qproj(0, wq_ref[0])
        qc_ref[...] = q0
        s0 = qk(q0, 0, 0)
        sc_ref[...] = s0
        mc_ref[...] = jnp.broadcast_to(jnp.max(s0[0:MROWS], axis=-1, keepdims=True), (MROWS, 128))

    for c in grp_b(h):
        c.wait()

    @pl.when(h + 1 < HKV)
    def _():
        for c in grp_a(h + 1):
            c.wait()
        for c in grp_b(h + 1):
            c.start()

    @pl.when(h + 2 < HKV)
    def _():
        for c in grp_a(h + 2):
            c.start()

    @pl.when(h == TR0)
    def _():
        all_chunks = wdt_ref.at[pl.ds(0, NFC)]
        pltpu.make_async_copy(all_chunks, all_chunks, sem_moe.at[2]).wait()
        for c in cp_up():
            c.start()

    @pl.when(h == TR0 + NFC)
    def _():
        for c in cp_up():
            c.wait()
        expert()

    attention_step()

    @pl.when(h == HKV - 1)
    def _epilogue():
        tl = NSUB - 1
        cols = slice(tl * TT, T)
        o_last = oc_ref[...]
        tail = []
        for b in range(NLAST):
            rows = slice(b * (DM // NLAST), (b + 1) * (DM // NLAST))
            s = acc_ref[rows, cols] + oproj(o_last, wot_ref[HKV - 1, rows, :])
            out_ref[rows, cols] = (xt_ref[rows, cols].astype(f32) + s * gt_ref[rows, cols]).astype(bf16)
            dst = (pl.ds(rows.start, DM // NLAST), pl.ds(tl * TT, TT))
            tail.append(pltpu.make_async_copy(out_ref.at[dst], out_hbm.at[dst], sem_out.at[tl + b]))
            tail[-1].start()
        for t in range(tl):
            cp_out(t).wait()
        for c in tail:
            c.wait()


@jax.jit
def pallas_recurrent_scan__gqa_block_cached__moe_arch_mod__prompt_kernel(
    A_x: jax.Array,
    A_k_cache: jax.Array,
    A_v_cache: jax.Array,
    A_wq: jax.Array,
    A_wo: jax.Array,
    B_x: jax.Array,
    B_w_r: jax.Array,
    B_w_gate: jax.Array,
    B_w_up: jax.Array,
    B_w_down: jax.Array,
):
    del B_x
    xt = A_x.reshape(T, DM).T
    k = A_k_cache.reshape(HKV, SK, DH)
    v = A_v_cache.reshape(HKV, SK, DH)
    wot = A_wo.T
    wdt = B_w_down.T
    hbm = pl.BlockSpec(memory_space=pl.ANY)
    dma = pltpu.SemaphoreType.DMA
    out_t = pl.pallas_call(
        _kernel,
        out_shape=jax.ShapeDtypeStruct((DM, T), bf16),
        grid=(HKV,),
        in_specs=[hbm] * 9,
        out_specs=hbm,
        scratch_shapes=[
            pltpu.VMEM((8 * PAD0, 128), f32),
            pltpu.VMEM((DM, T), bf16),
            pltpu.VMEM((HKV, SK, DH), bf16),
            pltpu.VMEM((HKV, SK, DH), bf16),
            pltpu.VMEM((HKV, DM, 2 * DH), bf16),
            pltpu.VMEM((HKV, DM, 2 * DH), bf16),
            pltpu.VMEM((T, DM), f32),
            pltpu.VMEM((DM, T), f32),
            pltpu.VMEM((DM, T), f32),
            pltpu.VMEM((DM, T), bf16),
            pltpu.VMEM((NFC + 1, DM, FC), bf16),
            pltpu.VMEM((FF + FC, DM), bf16),
            pltpu.VMEM((2 * TT, DH), bf16),
            pltpu.VMEM((2 * TT, CK), f32),
            pltpu.VMEM((MROWS, 128), f32),
            pltpu.VMEM((TT, 2 * DH), bf16),
            pltpu.VMEM((CAP, DM), f32),
            pltpu.VMEM((CAP, 128), f32),
            pltpu.SMEM((CAP,), jnp.int32),
            pltpu.VMEM((DM, FF), bf16),
            pltpu.VMEM((DM, FF), bf16),
            pltpu.VMEM((DM,), bf16),
            dma((len(PIECES),)), dma(()), dma((HKV,)), dma((HKV,)), dma((3,)), dma((NSUB - 1 + NLAST,)),
        ],
        compiler_params=pltpu.CompilerParams(
            dimension_semantics=("arbitrary",),
            disable_bounds_checks=True,
            vmem_limit_bytes=120 * 1024 * 1024,
        ),
    )(xt, k, v, A_wq, wot, B_w_r, B_w_gate, B_w_up, wdt)
    return out_t.T.reshape(1, T, DM)
```
